```python
import jax
import jax.numpy as jnp

def _softmax(x, axis=-1):
    return jax.nn.softmax(x, axis=axis)
def _gelu(x):
    return jax.nn.gelu(x, approximate=True)
def _silu(x):
    return jax.nn.silu(x)
def _sigmoid(x):
    return jax.nn.sigmoid(x)
def _layernorm(x, axis=-1, eps=1e-5):
    m = jnp.mean(x, axis=axis, keepdims=True)
    v = jnp.var(x, axis=axis, keepdims=True)
    return (x - m) / jnp.sqrt(v + eps)
def _scatter_add(tgt, idx, src, axis=0):
    return tgt.at[idx].add(src)
def _segment_sum(src, seg, n):
    return jax.ops.segment_sum(src, seg, n)
class _Rng:
    def __init__(self, key):
        self._k = key
    def _next(self):
        self._k, sub = jax.random.split(self._k)
        return sub
    def normal(self, shape):
        return jax.random.normal(self._next(), shape, dtype=jnp.bfloat16)
    def randint(self, lo, hi, shape):
        return jax.random.randint(self._next(), shape, lo, hi, dtype=jnp.int32)
    def uniform(self, shape, lo=0.0, hi=1.0):
        return jax.random.uniform(self._next(), shape, jnp.bfloat16, lo, hi)
    def permutation(self, n):
        return jax.random.permutation(self._next(), n)


kernel_name = 'standalone__self_sup_conv_stem_wavlm__speech'

def setup_inputs():
    _rng = _Rng(jax.random.key(int.from_bytes(__import__("os").urandom(4), "little")))
    _w = (lambda a: (lambda t: t.astype(jnp.bfloat16) if jnp.issubdtype(t.dtype, jnp.floating) else t)(jnp.asarray(a)))
    B, T, D, K = 2, 16000, 512, 31
    scale = (K * D) ** -0.5
    return {
        "x": _w((lambda *s: _rng.normal(s) * 0.05)(B, T, D)),
        "w": _w((lambda *s: _rng.normal(s) * 0.05)(K, D, D) * scale),
        "gn_gamma": _w((lambda *s: _rng.normal(s) * 0.05)(D) * 0.1 + 1.0),
        "gn_beta": _w((lambda *s: _rng.normal(s) * 0.05)(D) * 0.1),
    }

def reference(x, w, gn_gamma, gn_beta):
    B, T, D = x.shape
    K = w.shape[0]
    s = 2
    L = (T - K) // s + 1
    h = jnp.einsum('blc,cd->bld', x[:, 0:s * L:s, :], w[0])
    for i in range(1, K):
        h = h + jnp.einsum('blc,cd->bld', x[:, i:i + s * L:s, :], w[i])
    mu = jnp.einsum('bld->bd', h)[:, None, :] / L
    var = jnp.einsum('bld->bd', (h - mu) ** 2)[:, None, :] / L
    h = (h - mu) / jnp.sqrt(var + 1e-5)
    h = h * gn_gamma[None, None, :] + gn_beta[None, None, :]
    return _gelu(h)
```

```python
import jax
import jax.numpy as jnp
import jax.experimental.pallas as pl
import jax.experimental.pallas.tpu as pltpu

_TL = 512


def _gelu(x):
    c = 0.7978845608028654
    return 0.5 * x * (1.0 + jnp.tanh(c * (x + 0.044715 * (x * x * x))))


@jax.jit
def pallas_standalone__self_sup_conv_stem_wavlm__speech_kernel(
    x: jax.Array,
    w: jax.Array,
    gn_gamma: jax.Array,
    gn_beta: jax.Array,
):
    B, T, D = x.shape
    K = w.shape[0]
    L = (T - K) // 2 + 1
    U = T // 2
    u = x.reshape(B, U, 2 * D)
    nt = pl.cdiv(L, _TL)

    def kernel(u_ref, w_ref, g_ref, b_ref, o_ref, h_ref):
        def tile(i, carry):
            s1 = carry
            l0 = pl.multiple_of(jnp.minimum(i * _TL, U - _TL - 16), 16)
            ut = u_ref[pl.ds(l0, _TL + 16), :]
            acc = jnp.zeros((_TL, D), jnp.float32)
            for j in range(16):
                z = jnp.dot(ut[:, :D], w_ref[2 * j], preferred_element_type=jnp.float32)
                if 2 * j + 1 < K:
                    z = z + jnp.dot(ut[:, D:], w_ref[2 * j + 1], preferred_element_type=jnp.float32)
                acc = acc + z[j:j + _TL]
            h_ref[pl.ds(l0, _TL), :] = acc
            return s1

        jax.lax.fori_loop(0, nt, tile, 0)
        us = u_ref[U - 32:U, :]
        r = L - 1 - (U - 32)
        last = jnp.zeros((1, D), jnp.float32)
        for j in range(16):
            z = jnp.dot(us[:, :D], w_ref[2 * j], preferred_element_type=jnp.float32)
            if 2 * j + 1 < K:
                z = z + jnp.dot(us[:, D:], w_ref[2 * j + 1], preferred_element_type=jnp.float32)
            last = last + z[r + j:r + j + 1]
        h_ref[L - 1:L, :] = last

        def s_body(i, s):
            return s + jnp.sum(h_ref[pl.ds(i * 8, 8), :].reshape(1, 8, D), axis=0)
        n8 = L // 8
        def red(fn):
            def body(i, s):
                blk = h_ref[pl.ds(pl.multiple_of(i * 64, 64), 64), :]
                return s + jnp.sum(fn(blk).reshape(8, 8, D), axis=0)
            nb = (n8 * 8) // 64
            s = jax.lax.fori_loop(0, nb, body, jnp.zeros((8, D), jnp.float32))
            rem = h_ref[nb * 64:L, :]
            return jnp.sum(s, axis=0, keepdims=True) + jnp.sum(fn(rem), axis=0, keepdims=True)
        mu = red(lambda v: v) / L
        var = red(lambda v: (v - mu) * (v - mu)) / L
        rs = 1.0 / jnp.sqrt(var + 1e-5)
        g = g_ref[...].astype(jnp.float32)
        bb = b_ref[...].astype(jnp.float32)

        def fin(i, _):
            r0 = pl.multiple_of(i * 64, 64)
            blk = h_ref[pl.ds(r0, 64), :]
            y = (blk - mu) * rs * g + bb
            o_ref[pl.ds(r0, 64), :] = _gelu(y).astype(o_ref.dtype)
            return 0
        nb = L // 64
        jax.lax.fori_loop(0, nb, fin, 0)
        blk = h_ref[nb * 64:L, :]
        y = (blk - mu) * rs * g + bb
        o_ref[nb * 64:L, :] = _gelu(y).astype(o_ref.dtype)

    return pl.pallas_call(
        kernel,
        grid=(B,),
        in_specs=[
            pl.BlockSpec((None, U, 2 * D), lambda b: (b, 0, 0)),
            pl.BlockSpec((K, D, D), lambda b: (0, 0, 0), pipeline_mode=pl.Buffered(1)),
            pl.BlockSpec((1, D), lambda b: (0, 0)),
            pl.BlockSpec((1, D), lambda b: (0, 0)),
        ],
        out_specs=pl.BlockSpec((None, L, D), lambda b: (b, 0, 0)),
        out_shape=jax.ShapeDtypeStruct((B, L, D), x.dtype),
        scratch_shapes=[pltpu.VMEM((U, D), jnp.float32)],
        compiler_params=pltpu.CompilerParams(
            dimension_semantics=("arbitrary",),
            vmem_limit_bytes=120 * 1024 * 1024,
        ),
    )(u, w, gn_gamma.reshape(1, D), gn_beta.reshape(1, D))
```

```python
import functools
import numpy as np
import jax
import jax.numpy as jnp
import jax.experimental.pallas as pl
import jax.experimental.pallas.tpu as pltpu

_VARIANT = 'C'
_N = 64
_HOP = 48
_NS = 32


def _slot_freqs():
    return ([0] + [4 * k for k in range(1, 8)] + [4 * k + 2 for k in range(8)]
            + [2 * k + 1 for k in range(16)])


def _build_consts():
    n = _N
    th = 2 * np.pi / n
    fr = _slot_freqs()
    p = np.arange(16)

    def fwd_real(k):
        f = fr[k]
        if k == 0:
            return np.stack([np.ones(16), (-1.0) ** p])
        return np.stack([np.cos(th * f * p), -np.sin(th * f * p)])

    t02 = np.zeros((256, 128))
    t1 = np.zeros((256, 256))
    for kk in range(16):
        for cmp in range(2):
            for b in range(8):
                t02[16 * kk + 8 * cmp + b, 16 * b:16 * b + 16] = fwd_real(kk)[cmp]
    for kk in range(16):
        f = fr[16 + kk]
        c = np.cos(th * f * p)
        s = np.sin(th * f * p)
        if f % 4 == 1:
            re, im = (c, -s), (-s, -c)
        else:
            re, im = (c, s), (-s, c)
        for b in range(8):
            for part in range(2):
                c0 = 128 * part + 16 * b
                t1[16 * kk + b, c0:c0 + 16] = re[part]
                t1[16 * kk + 8 + b, c0:c0 + 16] = im[part]
    a02 = np.zeros((256, 128))
    a1 = np.zeros((256, 256))
    for kk in range(8):
        for b in range(8):
            f = fr[kk]
            if kk == 0:
                a02[16 * b:16 * b + 16, b] = 1.0 / n
                a02[16 * b:16 * b + 16, 8 + b] = (-1.0) ** p / n
            else:
                a02[16 * b:16 * b + 16, 16 * kk + b] = 2.0 / n * np.cos(th * f * p)
                a02[16 * b:16 * b + 16, 16 * kk + 8 + b] = -2.0 / n * np.sin(th * f * p)
            f = fr[8 + kk]
            a02[128 + 16 * b:128 + 16 * b + 16, 16 * kk + b] = 2.0 / n * np.cos(th * f * p)
            a02[128 + 16 * b:128 + 16 * b + 16, 16 * kk + 8 + b] = -2.0 / n * np.sin(th * f * p)
    for kk in range(16):
        f = fr[16 + kk]
        c = np.cos(th * f * p)
        s = np.sin(th * f * p)
        sg = -1.0 if f % 4 == 1 else 1.0
        for b in range(8):
            a1[16 * b:16 * b + 16, 16 * kk + b] = 2.0 / n * c
            a1[16 * b:16 * b + 16, 16 * kk + 8 + b] = -2.0 / n * s
            a1[128 + 16 * b:128 + 16 * b + 16, 16 * kk + b] = sg * 2.0 / n * s
            a1[128 + 16 * b:128 + 16 * b + 16, 16 * kk + 8 + b] = sg * 2.0 / n * c
    j = np.arange(16)
    g = np.zeros((64, 16))
    for k in range(32):
        f = fr[k]
        if k == 0:
            g[0] = 1.0
            g[1] = (-1.0) ** j
        else:
            g[2 * k] = np.cos(th * f * j)
            g[2 * k + 1] = np.sin(th * f * j)
    gk = np.zeros((512, 128))
    for m in range(64):
        for c in range(8):
            gk[8 * m + c, np.arange(16) * 8 + c] = g[m]
    bf = jnp.bfloat16
    return tuple(np.asarray(a, np.float32).astype(bf) for a in (t02, t1, a02, a1, gk))


_CONSTS = _build_consts()


def _gelu(x):
    c = 0.7978845608028654
    return 0.5 * x * (1.0 + jnp.tanh(c * (x + 0.044715 * (x * x * x))))


def _dot(a, b):
    return jnp.dot(a, b, preferred_element_type=jnp.float32)


@jax.jit
def pallas_standalone__self_sup_conv_stem_wavlm__speech_kernel(
    x: jax.Array,
    w: jax.Array,
    gn_gamma: jax.Array,
    gn_beta: jax.Array,
):
    B, T, D = x.shape
    K = w.shape[0]
    L = (T - K) // 2 + 1
    assert (T, D, K) == (16000, 512, 31)
    NG = 21
    GR = 8 * _HOP
    XR = 2 * (GR + 16)
    XPAD = 2 * GR * (NG - 1) + XR
    MR = 16 * NG
    GPC = 3
    CH = GPC * GR
    NCH = NG // GPC
    bf16, f32 = jnp.bfloat16, jnp.float32

    def kernel(x_hbm, w_hbm, g_ref, b_ref, t02_ref, t1_ref, a02_ref, a1_ref, gk_ref,
               o_ref, wf_ref, xb_ref, buf_ref, y_ref, st_ref, sh_ref, tmp_ref, xsem, wsem):
        step = pl.program_id(0)
        b = jnp.minimum(step, B - 1)

        def x_copy(bb):
            return pltpu.make_async_copy(x_hbm.at[bb], xb_ref.at[pl.ds(0, T)], xsem)

        def w_copy(i):
            return pltpu.make_async_copy(
                w_hbm.at[i], buf_ref.at[pl.ds(D * (i % 16), D), pl.ds(D * (i // 16), D)], wsem)

        def h_store(gi, hh):
            bits = pltpu.bitcast(hh, bf16)
            if isinstance(gi, int):
                buf_ref[2 * GR * (gi // 2):2 * GR * (gi // 2 + 1), D * (gi % 2):D * (gi % 2 + 1)] = bits
            else:
                r0 = pl.multiple_of((gi // 2) * (2 * GR), 2 * GR)
                c0 = pl.multiple_of((gi % 2) * D, D)
                buf_ref[pl.ds(r0, 2 * GR), pl.ds(c0, D)] = bits

        def h_load(gi):
            if isinstance(gi, int):
                bits = buf_ref[2 * GR * (gi // 2):2 * GR * (gi // 2 + 1), D * (gi % 2):D * (gi % 2 + 1)]
            else:
                r0 = pl.multiple_of((gi // 2) * (2 * GR), 2 * GR)
                c0 = pl.multiple_of((gi % 2) * D, D)
                bits = buf_ref[pl.ds(r0, 2 * GR), pl.ds(c0, D)]
            return pltpu.bitcast(bits, f32)

        @pl.when(step == 0)
        def _():
            for i in range(K):
                w_copy(i).start()
            x_copy(0).start()
            xb_ref[T:XPAD, :] = jnp.zeros((XPAD - T, D), bf16)
            for i in range(K):
                w_copy(i).wait()
            gk = gk_ref[...]
            for s in range(2):
                ntap = 16 if s == 0 else 15

                def body(ci, c):
                    c0 = pl.multiple_of(ci * 16, 16)
                    vs = []
                    for j in range(ntap):
                        i = 2 * j + s
                        vs.append(buf_ref[pl.ds(D * (i % 16) + c0, 16), D * (i // 16):D * (i // 16 + 1)].astype(f32))
                    res = []
                    for hh in range(2):
                        parts = [v[8 * hh:8 * hh + 8] for v in vs]
                        if ntap < 16:
                            parts.append(jnp.zeros((8, D), f32))
                        kt = jnp.concatenate(parts, axis=0).astype(bf16)
                        res.append(_dot(gk, kt))
                    r = jnp.concatenate([res[0].reshape(64, 8, D), res[1].reshape(64, 8, D)], axis=1)
                    r = r.astype(bf16)
                    for m in range(64):
                        wf_ref[m // 2, pl.ds(s * D + c0, 16), (m % 2) * D:(m % 2 + 1) * D] = r[m]
                    return c
                jax.lax.fori_loop(0, D // 16, body, 0)

        @pl.when(step < B)
        def _():
            x_copy(b).wait()

            def fwd(gi, c):
                r0 = pl.multiple_of(gi * (2 * GR), 2 * GR)
                xt = xb_ref[pl.ds(r0, XR), :]
                w32 = pltpu.bitcast(xt, jnp.uint32)
                for s in range(2):
                    if s == 0:
                        arr = pltpu.bitcast(w32 << 16, f32)
                    else:
                        arr = pltpu.bitcast(w32 & jnp.uint32(0xFFFF0000), f32)
                    tq = [jnp.concatenate([arr[16 * (3 * bb + q):16 * (3 * bb + q) + 16] for bb in range(8)], axis=0)
                          for q in range(4)]
                    e = tq[0] + tq[2]
                    o = tq[1] + tq[3]
                    z0 = (e + o).astype(bf16)
                    z2 = (e - o).astype(bf16)
                    za = (tq[0] - tq[2]).astype(bf16)
                    zb = (tq[1] - tq[3]).astype(bf16)
                    x0 = _dot(t02_ref[0:128, :], z0).astype(bf16)
                    x2 = _dot(t02_ref[128:256, :], z2).astype(bf16)
                    x1 = _dot(t1_ref[...], jnp.concatenate([za, zb], axis=0)).astype(bf16)
                    for kk in range(8):
                        buf_ref[pl.ds(kk * MR + gi * 16, 16), s * D:(s + 1) * D] = x0[16 * kk:16 * kk + 16]
                        buf_ref[pl.ds((8 + kk) * MR + gi * 16, 16), s * D:(s + 1) * D] = x2[16 * kk:16 * kk + 16]
                    for kk in range(16):
                        buf_ref[pl.ds((16 + kk) * MR + gi * 16, 16), s * D:(s + 1) * D] = x1[16 * kk:16 * kk + 16]
                return c
            jax.lax.fori_loop(0, NG, fwd, 0)

            @pl.when(b + 1 < B)
            def _():
                x_copy(b + 1).start()

            def mix(k, special):
                if special:
                    xs = buf_ref[0:MR, :]
                else:
                    xs = buf_ref[pl.ds(pl.multiple_of(k * MR, 16), MR), :]
                p = _dot(xs, wf_ref[k]).reshape(NG, 2, 8, 2 * D)
                pa = p[:, 0]
                pb = p[:, 1]
                if special:
                    yr = pa[:, :, :D]
                    yi = pb[:, :, D:]
                else:
                    yr = pa[:, :, :D] - pb[:, :, D:]
                    yi = pa[:, :, D:] + pb[:, :, :D]
                y = jnp.concatenate([yr, yi], axis=1).reshape(MR, D)
                y_ref[k] = y.astype(bf16)
            mix(0, True)

            def mbody(k, c):
                mix(k, False)
                return c
            jax.lax.fori_loop(1, _NS, mbody, 0)

            def inv(gi, s1, last):
                m0 = gi * 16 if last else pl.multiple_of(gi * 16, 16)
                y0 = jnp.concatenate([y_ref[kk, pl.ds(m0, 16), :] for kk in range(8)], axis=0)
                y2 = jnp.concatenate([y_ref[8 + kk, pl.ds(m0, 16), :] for kk in range(8)], axis=0)
                y1 = jnp.concatenate([y_ref[16 + kk, pl.ds(m0, 16), :] for kk in range(16)], axis=0)
                z0 = _dot(a02_ref[0:128, :], y0).reshape(8, 16, D)
                z2 = _dot(a02_ref[128:256, :], y2).reshape(8, 16, D)
                ab = _dot(a1_ref[...], y1)
                za = ab[:128].reshape(8, 16, D)
                zb = ab[128:].reshape(8, 16, D)
                e = z0 + z2
                hh = jnp.concatenate([e + za, (z0 - z2) + zb, e - za], axis=1).reshape(GR, D)
                if last:
                    row = jax.lax.broadcasted_iota(jnp.int32, (GR, D), 0)
                    hh = jnp.where(row < L - GR * (NG - 1), hh, 0.0)
                h_store(gi, hh)
                return s1 + jnp.sum(hh.reshape(GR // 8, 8, D), axis=0)
            s1 = jax.lax.fori_loop(0, NG - 1, lambda gi, s: inv(gi, s, False), jnp.zeros((8, D), f32))
            s1 = inv(NG - 1, s1, True)
            mu = jnp.sum(s1, axis=0, keepdims=True) * (1.0 / L)

            def vbody(gi, s2):
                hh = h_load(gi) - mu
                return s2 + jnp.sum((hh * hh).reshape(GR // 8, 8, D), axis=0)
            s2 = jax.lax.fori_loop(0, NG - 1, vbody, jnp.zeros((8, D), f32))
            hh = h_load(NG - 1) - mu
            row = jax.lax.broadcasted_iota(jnp.int32, (GR, D), 0)
            hh = jnp.where(row < L - GR * (NG - 1), hh, 0.0)
            s2 = s2 + jnp.sum((hh * hh).reshape(GR // 8, 8, D), axis=0)
            var = jnp.sum(s2, axis=0, keepdims=True) * (1.0 / L)
            st_ref[0:1, :] = mu
            st_ref[1:2, :] = g_ref[...].astype(f32) / jnp.sqrt(var + 1e-5)

        def act(gi):
            mu = st_ref[0:1, :]
            scale = st_ref[1:2, :]
            beta = b_ref[...].astype(f32)
            hh = h_load(gi)
            return _gelu((hh - mu) * scale + beta)

        @pl.when(step == 0)
        def _():
            def fin0(gi, c):
                sh_ref[pl.ds(pl.multiple_of(gi * GR, GR), GR), :] = act(gi).astype(bf16)
                return c
            jax.lax.fori_loop(0, NG, fin0, 0)

        @pl.when(step >= B)
        def _():
            def fin(j, c):
                gi = (step - B) * GPC + j
                y1 = act(gi)
                y0 = sh_ref[pl.ds(pl.multiple_of(gi * GR, GR), GR), :]
                if _VARIANT == 'A':
                    o_ref[pl.ds(pl.multiple_of(j * GR, GR), GR)] = jnp.stack([y0.astype(f32), y1], axis=1).astype(bf16)
                else:
                    lo = pltpu.bitcast(y0.astype(f32), jnp.uint32) >> 16
                    hi = pltpu.bitcast(y1.astype(bf16).astype(f32), jnp.uint32)
                    wv = lo | hi
                    for cc in range(4):
                        tmp_ref[pl.ds(cc, GR, stride=4), :] = wv[:, 128 * cc:128 * (cc + 1)]
                    o_ref[pl.ds(pl.multiple_of(j * 8 * GR, 8 * GR), 8 * GR), :] = pltpu.bitcast(tmp_ref[...], bf16)
                return c
            jax.lax.fori_loop(0, GPC, fin, 0)

    vm = lambda shape: pl.BlockSpec(shape, lambda s: (0,) * len(shape))
    any_spec = pl.BlockSpec(memory_space=pl.ANY)
    out = pl.pallas_call(
        kernel,
        grid=(B + NCH,),
        in_specs=[any_spec, any_spec, vm((1, D)), vm((1, D)),
                  vm((256, 128)), vm((256, 256)), vm((256, 128)), vm((256, 256)), vm((512, 128))],
        out_specs=(pl.BlockSpec((CH, B, D), lambda s: (jnp.maximum(s - B, 0), 0, 0)) if _VARIANT == 'A'
                   else pl.BlockSpec((CH * 8, 128), lambda s: (jnp.maximum(s - B, 0), 0))),
        out_shape=(jax.ShapeDtypeStruct((L, B, D), x.dtype) if _VARIANT == 'A'
                   else jax.ShapeDtypeStruct((L * 8, 128), x.dtype)),
        scratch_shapes=[
            pltpu.VMEM((_NS, 2 * D, 2 * D), bf16),
            pltpu.VMEM((XPAD, D), bf16),
            pltpu.VMEM((_NS * MR, 2 * D), bf16),
            pltpu.VMEM((_NS, MR, D), bf16),
            pltpu.VMEM((8, D), f32),
            pltpu.VMEM((NG * GR, D), bf16),
            pltpu.VMEM((4 * GR, 128), jnp.uint32) if _VARIANT != 'A' else pltpu.VMEM((8, 128), jnp.uint32),
            pltpu.SemaphoreType.DMA(()),
            pltpu.SemaphoreType.DMA(()),
        ],
        compiler_params=pltpu.CompilerParams(
            dimension_semantics=("arbitrary",),
            vmem_limit_bytes=128 * 1024 * 1024,
        ),
    )(x, w, gn_gamma.reshape(1, D), gn_beta.reshape(1, D), *_CONSTS)
    if _VARIANT == 'A':
        return out.transpose(1, 0, 2)
    return out.reshape(L, 4, B, 128).transpose(2, 0, 1, 3).reshape(B, L, D)
```

```python
import functools
import numpy as np
import jax
import jax.numpy as jnp
import jax.experimental.pallas as pl
import jax.experimental.pallas.tpu as pltpu

_N = 64
_HOP = 48
_NS = 32


def _slot_freqs():
    return ([0] + [4 * k for k in range(1, 8)] + [4 * k + 2 for k in range(8)]
            + [2 * k + 1 for k in range(16)])


def _build_consts():
    n = _N
    th = 2 * np.pi / n
    fr = _slot_freqs()
    p = np.arange(16)

    def fwd_real(k):
        f = fr[k]
        if k == 0:
            return np.stack([np.ones(16), (-1.0) ** p])
        return np.stack([np.cos(th * f * p), -np.sin(th * f * p)])

    t02 = np.zeros((256, 128))
    t1 = np.zeros((256, 256))
    for kk in range(16):
        for cmp in range(2):
            for b in range(8):
                t02[16 * kk + 2 * b + cmp, 16 * b:16 * b + 16] = fwd_real(kk)[cmp]
    for kk in range(16):
        f = fr[16 + kk]
        c = np.cos(th * f * p)
        s = np.sin(th * f * p)
        if f % 4 == 1:
            re, im = (c, -s), (-s, -c)
        else:
            re, im = (c, s), (-s, c)
        for b in range(8):
            for part in range(2):
                c0 = 128 * part + 16 * b
                t1[16 * kk + 2 * b, c0:c0 + 16] = re[part]
                t1[16 * kk + 2 * b + 1, c0:c0 + 16] = im[part]
    a02 = np.zeros((256, 128))
    a1 = np.zeros((256, 256))
    for kk in range(8):
        for b in range(8):
            f = fr[kk]
            if kk == 0:
                a02[16 * b:16 * b + 16, b] = 1.0 / n
                a02[16 * b:16 * b + 16, 8 + b] = (-1.0) ** p / n
            else:
                a02[16 * b:16 * b + 16, 16 * kk + b] = 2.0 / n * np.cos(th * f * p)
                a02[16 * b:16 * b + 16, 16 * kk + 8 + b] = -2.0 / n * np.sin(th * f * p)
            f = fr[8 + kk]
            a02[128 + 16 * b:128 + 16 * b + 16, 16 * kk + b] = 2.0 / n * np.cos(th * f * p)
            a02[128 + 16 * b:128 + 16 * b + 16, 16 * kk + 8 + b] = -2.0 / n * np.sin(th * f * p)
    for kk in range(16):
        f = fr[16 + kk]
        c = np.cos(th * f * p)
        s = np.sin(th * f * p)
        sg = -1.0 if f % 4 == 1 else 1.0
        for b in range(8):
            a1[16 * b:16 * b + 16, 16 * kk + b] = 2.0 / n * c
            a1[16 * b:16 * b + 16, 16 * kk + 8 + b] = -2.0 / n * s
            a1[128 + 16 * b:128 + 16 * b + 16, 16 * kk + b] = sg * 2.0 / n * s
            a1[128 + 16 * b:128 + 16 * b + 16, 16 * kk + 8 + b] = sg * 2.0 / n * c
    j = np.arange(16)
    g = np.zeros((64, 16))
    for k in range(32):
        f = fr[k]
        if k == 0:
            g[0] = 1.0
            g[1] = (-1.0) ** j
        else:
            g[2 * k] = np.cos(th * f * j)
            g[2 * k + 1] = np.sin(th * f * j)
    gk = np.zeros((512, 128))
    for m in range(64):
        for c in range(8):
            gk[8 * m + c, np.arange(16) * 8 + c] = g[m]
    pm = np.zeros((128, 128))
    for bb in range(2):
        for ct in range(4):
            for l in range(16):
                pm[l * 8 + ct * 2 + bb, (bb * 4 + ct) * 16 + l] = 1.0
    bf = jnp.bfloat16
    return tuple(np.asarray(a, np.float32).astype(bf) for a in (t02, t1, a02, a1, gk, pm))


_CONSTS = _build_consts()


def _gelu(x):
    c = 0.7978845608028654
    return 0.5 * x * (1.0 + jnp.tanh(c * (x + 0.044715 * (x * x * x))))


def _dot(a, b):
    return jnp.dot(a, b, preferred_element_type=jnp.float32)


@jax.jit
def pallas_standalone__self_sup_conv_stem_wavlm__speech_kernel(
    x: jax.Array,
    w: jax.Array,
    gn_gamma: jax.Array,
    gn_beta: jax.Array,
):
    B, T, D = x.shape
    K = w.shape[0]
    L = (T - K) // 2 + 1
    assert (T, D, K) == (16000, 512, 31)
    NG = 21
    GR = 8 * _HOP
    XR = 2 * (GR + 16)
    XPAD = 2 * GR * (NG - 1) + XR
    MR = 16 * NG
    WC = 64
    NWC = D // WC
    NWS = 5
    GPC = 3
    CH = GPC * GR
    NCH = NG // GPC
    bf16, f32 = jnp.bfloat16, jnp.float32

    def kernel(x_hbm, w_hbm, g_ref, b_ref, t02_ref, t1_ref, a02_ref, a1_ref, gk_ref, pm_ref,
               o_ref, wf_ref, xb_ref, buf_ref, y_ref, st_ref, sh_ref, xsem, wsem):
        step = pl.program_id(0)
        b = jnp.minimum(step, B - 1)

        def x_copy(bb):
            return pltpu.make_async_copy(x_hbm.at[bb], xb_ref.at[pl.ds(0, T)], xsem)

        def x_piece(i):
            n = T // NWC
            return pltpu.make_async_copy(x_hbm.at[0, pl.ds(i * n, n)], xb_ref.at[pl.ds(i * n, n)], xsem)

        def w_copy(ch):
            slot = ch % NWS
            return pltpu.make_async_copy(
                w_hbm.at[:, pl.ds(ch * WC, WC), :], y_ref.at[pl.ds(0, K), pl.ds(slot * WC, WC), :], wsem.at[slot])

        def h_store(gi, hh):
            bits = pltpu.bitcast(hh, bf16)
            if isinstance(gi, int):
                buf_ref[2 * GR * (gi // 2):2 * GR * (gi // 2 + 1), D * (gi % 2):D * (gi % 2 + 1)] = bits
            else:
                r0 = pl.multiple_of((gi // 2) * (2 * GR), 2 * GR)
                c0 = pl.multiple_of((gi % 2) * D, D)
                buf_ref[pl.ds(r0, 2 * GR), pl.ds(c0, D)] = bits

        def h_load(gi):
            if isinstance(gi, int):
                bits = buf_ref[2 * GR * (gi // 2):2 * GR * (gi // 2 + 1), D * (gi % 2):D * (gi % 2 + 1)]
            else:
                r0 = pl.multiple_of((gi // 2) * (2 * GR), 2 * GR)
                c0 = pl.multiple_of((gi % 2) * D, D)
                bits = buf_ref[pl.ds(r0, 2 * GR), pl.ds(c0, D)]
            return pltpu.bitcast(bits, f32)

        @pl.when(step == 0)
        def _():
            for ch in range(2):
                w_copy(ch).start()
            xb_ref[T:XPAD, :] = jnp.zeros((XPAD - T, D), bf16)
            gk = gk_ref[...]

            def wchunk(ch, c):
                w_copy(ch).wait()

                @pl.when(ch + 2 < NWC)
                def _():
                    w_copy(ch + 2).start()
                x_piece(ch).start()
                r0 = pl.multiple_of((ch % NWS) * WC, WC)
                for s in range(2):
                    ntap = 16 if s == 0 else 15

                    def body(ci, c):
                        c0 = pl.multiple_of(ci * 16, 16)
                        vs = [y_ref[2 * j + s, pl.ds(r0 + c0, 16), :].astype(f32) for j in range(ntap)]
                        res = []
                        for hh in range(2):
                            parts = [v[8 * hh:8 * hh + 8] for v in vs]
                            if ntap < 16:
                                parts.append(jnp.zeros((8, D), f32))
                            kt = jnp.concatenate(parts, axis=0).astype(bf16)
                            res.append(_dot(gk, kt))
                        r = jnp.concatenate([res[0].reshape(64, 8, D), res[1].reshape(64, 8, D)], axis=1)
                        r = r.astype(bf16)
                        cw = pl.multiple_of(s * D + ch * WC + c0, 16)
                        for m in range(64):
                            wf_ref[m // 2, pl.ds(cw, 16), (m % 2) * D:(m % 2 + 1) * D] = r[m]
                        return c
                    jax.lax.fori_loop(0, WC // 16, body, 0, unroll=4)
                return c
            jax.lax.fori_loop(0, NWC, wchunk, 0)

        @pl.when(step < B)
        def _():
            @pl.when(step == 0)
            def _():
                for i in range(NWC):
                    x_piece(i).wait()

            @pl.when(step > 0)
            def _():
                x_copy(b).wait()

            def fwd(gi, c):
                r0 = pl.multiple_of(gi * (2 * GR), 2 * GR)
                for s in range(2):
                    def tile(tt):
                        w32 = pltpu.bitcast(xb_ref[pl.ds(r0 + 32 * tt, 32), :], jnp.uint32)
                        if s == 0:
                            return pltpu.bitcast(w32 << 16, f32)
                        return pltpu.bitcast(w32 & jnp.uint32(0xFFFF0000), f32)
                    zs = [[], [], [], []]
                    t0 = tile(0)
                    for bb in range(8):
                        tb, tc, td = tile(3 * bb + 1), tile(3 * bb + 2), tile(3 * bb + 3)
                        e = t0 + tc
                        o = tb + td
                        zs[0].append((e + o).astype(bf16))
                        zs[1].append((e - o).astype(bf16))
                        zs[2].append((t0 - tc).astype(bf16))
                        zs[3].append((tb - td).astype(bf16))
                        t0 = td
                    z0, z2, za, zb = [jnp.concatenate(z, axis=0) for z in zs]
                    x0 = _dot(t02_ref[0:128, :], z0).astype(bf16)
                    x2 = _dot(t02_ref[128:256, :], z2).astype(bf16)
                    x1 = _dot(t1_ref[...], jnp.concatenate([za, zb], axis=0)).astype(bf16)
                    for kk in range(8):
                        buf_ref[pl.ds(kk * MR + gi * 16, 16), s * D:(s + 1) * D] = x0[16 * kk:16 * kk + 16]
                        buf_ref[pl.ds((8 + kk) * MR + gi * 16, 16), s * D:(s + 1) * D] = x2[16 * kk:16 * kk + 16]
                    for kk in range(16):
                        buf_ref[pl.ds((16 + kk) * MR + gi * 16, 16), s * D:(s + 1) * D] = x1[16 * kk:16 * kk + 16]
                return c
            jax.lax.fori_loop(0, NG, fwd, 0, unroll=3)

            @pl.when(b + 1 < B)
            def _():
                x_copy(b + 1).start()

            def mix(k, special):
                if special:
                    xs = buf_ref[0:MR, :]
                else:
                    xs = buf_ref[pl.ds(pl.multiple_of(k * MR, 16), MR), :]
                w32 = pltpu.bitcast(xs, jnp.uint32)
                xa = pltpu.bitcast(w32 << 16, f32)
                xi = pltpu.bitcast(w32 & jnp.uint32(0xFFFF0000), f32)
                wc = wf_ref[k, :, 0:D]
                wd = wf_ref[k, :, D:2 * D]
                t1 = _dot(xa.astype(bf16), wc)
                t2 = _dot(xi.astype(bf16), wd)
                if special:
                    yr, yi = t1, t2
                else:
                    we = (wc.astype(f32) + wd.astype(f32)).astype(bf16)
                    t3 = _dot((xa + xi).astype(bf16), we)
                    yr = t1 - t2
                    yi = t3 - (t1 + t2)
                y = jnp.concatenate([yr.reshape(NG, 8, D), yi.reshape(NG, 8, D)], axis=1).reshape(MR, D)
                y_ref[k] = y.astype(bf16)
            mix(0, True)

            def mbody(k, c):
                mix(k, False)
                return c
            jax.lax.fori_loop(1, _NS, mbody, 0, unroll=2)

            def inv(gi):
                m0 = gi * 16 if isinstance(gi, int) else pl.multiple_of(gi * 16, 16)
                y0 = jnp.concatenate([y_ref[kk, pl.ds(m0, 16), :] for kk in range(8)], axis=0)
                y2 = jnp.concatenate([y_ref[8 + kk, pl.ds(m0, 16), :] for kk in range(8)], axis=0)
                y1 = jnp.concatenate([y_ref[16 + kk, pl.ds(m0, 16), :] for kk in range(16)], axis=0)
                z0 = _dot(a02_ref[0:128, :], y0).reshape(8, 16, D)
                z2 = _dot(a02_ref[128:256, :], y2).reshape(8, 16, D)
                ab = _dot(a1_ref[...], y1)
                za = ab[:128].reshape(8, 16, D)
                zb = ab[128:].reshape(8, 16, D)
                e = z0 + z2
                hh = jnp.concatenate([e + za, (z0 - z2) + zb, e - za], axis=1).reshape(GR, D)
                h_store(gi, hh)
                return hh

            def acc(hh, sh, s1, s2):
                d = (hh - sh).reshape(GR // 8, 8, D)
                return s1 + jnp.sum(d, axis=0), s2 + jnp.sum(d * d, axis=0)

            h0 = inv(0)
            sh = jnp.sum(jnp.sum(h0.reshape(GR // 8, 8, D), axis=0), axis=0, keepdims=True) * (1.0 / GR)
            zz = jnp.zeros((8, D), f32)
            s1, s2 = acc(h0, sh, zz, zz)
            s1, s2 = jax.lax.fori_loop(1, NG - 1, lambda gi, c: acc(inv(gi), sh, *c), (s1, s2), unroll=3)
            hl = inv(NG - 1)
            row = jax.lax.broadcasted_iota(jnp.int32, (GR, D), 0)
            d = jnp.where(row < L - GR * (NG - 1), hl - sh, 0.0).reshape(GR // 8, 8, D)
            s1 = s1 + jnp.sum(d, axis=0)
            s2 = s2 + jnp.sum(d * d, axis=0)
            dm = jnp.sum(s1, axis=0, keepdims=True) * (1.0 / L)
            mu = sh + dm
            var = jnp.maximum(jnp.sum(s2, axis=0, keepdims=True) * (1.0 / L) - dm * dm, 0.0)
            st_ref[0:1, :] = mu
            st_ref[1:2, :] = g_ref[...].astype(f32) / jnp.sqrt(var + 1e-5)

        def act(gi):
            mu = st_ref[0:1, :]
            scale = st_ref[1:2, :]
            beta = b_ref[...].astype(f32)
            hh = h_load(gi)
            return _gelu((hh - mu) * scale + beta)

        @pl.when(step == 0)
        def _():
            def fin0(gi, c):
                sh_ref[pl.ds(pl.multiple_of(gi * GR, GR), GR), :] = act(gi).astype(bf16)
                return c
            jax.lax.fori_loop(0, NG, fin0, 0)

        @pl.when(step >= B)
        def _():
            def fin(j, c):
                gi = (step - B) * GPC + j
                y1 = act(gi)
                y0 = sh_ref[pl.ds(pl.multiple_of(gi * GR, GR), GR), :]
                y1b = y1.astype(bf16)
                cols = []
                for jj in range(GR // 16):
                    cols.append(jnp.concatenate(
                        [yy[16 * jj:16 * jj + 16, 128 * cc:128 * (cc + 1)] for yy in (y0, y1b) for cc in range(4)], axis=0))
                sm = jnp.concatenate(cols, axis=1)
                r = _dot(pm_ref[...], sm)
                rr = jnp.concatenate([r[:, 128 * jj:128 * (jj + 1)] for jj in range(GR // 16)], axis=0)
                o_ref[pl.ds(pl.multiple_of(j * 8 * GR, 8 * GR), 8 * GR), :] = rr.astype(bf16)
                return c
            jax.lax.fori_loop(0, GPC, fin, 0, unroll=3)

    vm = lambda shape: pl.BlockSpec(shape, lambda s: (0,) * len(shape))
    any_spec = pl.BlockSpec(memory_space=pl.ANY)
    out = pl.pallas_call(
        kernel,
        grid=(B + NCH,),
        in_specs=[any_spec, any_spec, vm((1, D)), vm((1, D)),
                  vm((256, 128)), vm((256, 256)), vm((256, 128)), vm((256, 256)), vm((512, 128)), vm((128, 128))],
        out_specs=pl.BlockSpec((CH * 8, 128), lambda s: (jnp.maximum(s - B, 0), 0)),
        out_shape=jax.ShapeDtypeStruct((L * 8, 128), x.dtype),
        scratch_shapes=[
            pltpu.VMEM((_NS, 2 * D, 2 * D), bf16),
            pltpu.VMEM((XPAD, D), bf16),
            pltpu.VMEM((_NS * MR, 2 * D), bf16),
            pltpu.VMEM((_NS, MR, D), bf16),
            pltpu.VMEM((8, D), f32),
            pltpu.VMEM((NG * GR, D), bf16),
            pltpu.SemaphoreType.DMA(()),
            pltpu.SemaphoreType.DMA((NWS,)),
        ],
        compiler_params=pltpu.CompilerParams(
            dimension_semantics=("arbitrary",),
            vmem_limit_bytes=128 * 1024 * 1024,
        ),
    )(x, w, gn_gamma.reshape(1, D), gn_beta.reshape(1, D), *_CONSTS)
    return out.reshape(L, 4, B, 128).transpose(2, 0, 1, 3).reshape(B, L, D)
```

```python
import functools
import numpy as np
import jax
import jax.numpy as jnp
import jax.experimental.pallas as pl
import jax.experimental.pallas.tpu as pltpu

_N = 64
_HOP = 48
_NS = 32


def _slot_freqs():
    return ([0] + [4 * k for k in range(1, 8)] + [4 * k + 2 for k in range(8)]
            + [2 * k + 1 for k in range(16)])


def _build_consts():
    n = _N
    th = 2 * np.pi / n
    fr = _slot_freqs()
    p = np.arange(16)

    def fwd_real(k):
        f = fr[k]
        if k == 0:
            return np.stack([np.ones(16), (-1.0) ** p])
        return np.stack([np.cos(th * f * p), -np.sin(th * f * p)])

    t02 = np.zeros((256, 128))
    t1 = np.zeros((256, 256))
    for kk in range(16):
        for cmp in range(2):
            for b in range(8):
                t02[16 * kk + 8 * cmp + b, 16 * b:16 * b + 16] = fwd_real(kk)[cmp]
    for kk in range(16):
        f = fr[16 + kk]
        c = np.cos(th * f * p)
        s = np.sin(th * f * p)
        if f % 4 == 1:
            re, im = (c, -s), (-s, -c)
        else:
            re, im = (c, s), (-s, c)
        for b in range(8):
            for part in range(2):
                c0 = 128 * part + 16 * b
                t1[16 * kk + b, c0:c0 + 16] = re[part]
                t1[16 * kk + 8 + b, c0:c0 + 16] = im[part]
    a02 = np.zeros((256, 128))
    a1 = np.zeros((256, 256))
    for kk in range(8):
        for b in range(8):
            f = fr[kk]
            if kk == 0:
                a02[16 * b:16 * b + 16, b] = 1.0 / n
                a02[16 * b:16 * b + 16, 8 + b] = (-1.0) ** p / n
            else:
                a02[16 * b:16 * b + 16, 16 * kk + b] = 2.0 / n * np.cos(th * f * p)
                a02[16 * b:16 * b + 16, 16 * kk + 8 + b] = -2.0 / n * np.sin(th * f * p)
            f = fr[8 + kk]
            a02[128 + 16 * b:128 + 16 * b + 16, 16 * kk + b] = 2.0 / n * np.cos(th * f * p)
            a02[128 + 16 * b:128 + 16 * b + 16, 16 * kk + 8 + b] = -2.0 / n * np.sin(th * f * p)
    for kk in range(16):
        f = fr[16 + kk]
        c = np.cos(th * f * p)
        s = np.sin(th * f * p)
        sg = -1.0 if f % 4 == 1 else 1.0
        for b in range(8):
            a1[16 * b:16 * b + 16, 16 * kk + b] = 2.0 / n * c
            a1[16 * b:16 * b + 16, 16 * kk + 8 + b] = -2.0 / n * s
            a1[128 + 16 * b:128 + 16 * b + 16, 16 * kk + b] = sg * 2.0 / n * s
            a1[128 + 16 * b:128 + 16 * b + 16, 16 * kk + 8 + b] = sg * 2.0 / n * c
    j = np.arange(16)
    g = np.zeros((64, 16))
    for k in range(32):
        f = fr[k]
        if k == 0:
            g[0] = 1.0
            g[1] = (-1.0) ** j
        else:
            g[2 * k] = np.cos(th * f * j)
            g[2 * k + 1] = np.sin(th * f * j)
    gk = np.zeros((512, 128))
    for m in range(64):
        for c in range(8):
            gk[8 * m + c, np.arange(16) * 8 + c] = g[m]
    pm = np.zeros((128, 128))
    for bb in range(2):
        for ct in range(4):
            for l in range(16):
                pm[l * 8 + ct * 2 + bb, (bb * 4 + ct) * 16 + l] = 1.0
    bf = jnp.bfloat16
    return tuple(np.asarray(a, np.float32).astype(bf) for a in (t02, t1, a02, a1, gk, pm))


_CONSTS = _build_consts()


def _gelu(x):
    c = 0.7978845608028654
    hx = 0.5 * x
    return hx + hx * jnp.tanh(x * (c + (c * 0.044715) * (x * x)))


def _pair(lo, hi):
    return pltpu.pack_elementwise([lo, hi], packed_dtype=jnp.bfloat16).astype(jnp.uint32)


def _part(w32, i):
    return pltpu.unpack_elementwise(w32, index=i, packed_dtype=jnp.bfloat16, unpacked_dtype=jnp.float32)


def _dot(a, b):
    return jnp.dot(a, b, preferred_element_type=jnp.float32)


@jax.jit
def pallas_standalone__self_sup_conv_stem_wavlm__speech_kernel(
    x: jax.Array,
    w: jax.Array,
    gn_gamma: jax.Array,
    gn_beta: jax.Array,
):
    B, T, D = x.shape
    K = w.shape[0]
    L = (T - K) // 2 + 1
    assert (T, D, K) == (16000, 512, 31)
    NG = 21
    GR = 8 * _HOP
    XR = 2 * (GR + 16)
    XPAD = 2 * GR * (NG - 1) + XR
    NW = 8 * NG
    MR = 16 * NG
    WC = 64
    NWC = D // WC
    NWS = 5
    GPC = 1
    CH = GPC * GR
    NCH = NG // GPC
    bf16, f32 = jnp.bfloat16, jnp.float32

    def kernel(x_hbm, w_hbm, g_ref, b_ref, t02_ref, t1_ref, a02_ref, a1_ref, gk_ref, pm_ref,
               o_ref, wf_ref, xb_ref, buf_ref, y_ref, st_ref, sh_ref, xsem, wsem):
        step = pl.program_id(0)
        b = jnp.minimum(step, B - 1)

        def x_copy(bb):
            return pltpu.make_async_copy(x_hbm.at[bb], xb_ref.at[pl.ds(0, T)], xsem)

        def x_piece(i):
            n = T // NWC
            return pltpu.make_async_copy(x_hbm.at[0, pl.ds(i * n, n)], xb_ref.at[pl.ds(i * n, n)], xsem)

        def w_copy(ch):
            slot = ch % NWS
            return pltpu.make_async_copy(
                w_hbm.at[:, pl.ds(ch * WC, WC), :], y_ref.at[pl.ds(0, K), pl.ds(slot * WC, WC), :], wsem.at[slot])

        def h_idx(gi):
            if isinstance(gi, int):
                return (pl.ds(GR * (gi // 2), GR), pl.ds(D * (gi % 2), D))
            return (pl.ds(pl.multiple_of((gi // 2) * GR, GR), GR), pl.ds(pl.multiple_of((gi % 2) * D, D), D))

        def h_store(gi, hh):
            buf_ref[h_idx(gi)] = pltpu.bitcast(hh, jnp.uint32)

        def finish(hh, row):
            scale = st_ref[row:row + 1, :]
            shift = st_ref[row + 1:row + 2, :]
            return _gelu(hh * scale + shift)

        @pl.when(step == 0)
        def _():
            for ch in range(2):
                w_copy(ch).start()
            xb_ref[T:XPAD, :] = jnp.zeros((XPAD - T, D), bf16)
            gk = gk_ref[...]

            def wchunk(ch, c):
                w_copy(ch).wait()

                @pl.when(ch + 2 < NWC)
                def _():
                    w_copy(ch + 2).start()
                x_piece(ch).start()
                r0 = pl.multiple_of((ch % NWS) * WC, WC)
                for s in range(2):
                    ntap = 16 if s == 0 else 15

                    def body(ci, c):
                        c0 = pl.multiple_of(ci * 16, 16)
                        vs = [y_ref[2 * j + s, pl.ds(r0 + c0, 16), :].astype(f32) for j in range(ntap)]
                        res = []
                        for hh in range(2):
                            parts = [v[8 * hh:8 * hh + 8] for v in vs]
                            if ntap < 16:
                                parts.append(jnp.zeros((8, D), f32))
                            kt = jnp.concatenate(parts, axis=0).astype(bf16)
                            res.append(_dot(gk, kt))
                        r = jnp.concatenate([res[0].reshape(64, 8, D), res[1].reshape(64, 8, D)], axis=1)
                        r = r.astype(bf16)
                        cw = pl.multiple_of(s * D + ch * WC + c0, 16)
                        for m in range(64):
                            wf_ref[m // 2, pl.ds(cw, 16), (m % 2) * D:(m % 2 + 1) * D] = r[m]
                        return c
                    jax.lax.fori_loop(0, WC // 16, body, 0, unroll=4)
                return c
            jax.lax.fori_loop(0, NWC, wchunk, 0)

        @pl.when(step < B)
        def _():
            @pl.when(step == 0)
            def _():
                for i in range(NWC):
                    x_piece(i).wait()

            @pl.when(step > 0)
            def _():
                x_copy(b).wait()

            def fwd(gi, c):
                r0 = pl.multiple_of(gi * (2 * GR), 2 * GR)
                for s in range(2):
                    def tile(tt):
                        w32 = pltpu.bitcast(xb_ref[pl.ds(r0 + 32 * tt, 32), :], jnp.uint32)
                        return _part(w32, s)
                    zs = [[], [], [], []]
                    t0 = tile(0)
                    for bb in range(8):
                        tb, tc, td = tile(3 * bb + 1), tile(3 * bb + 2), tile(3 * bb + 3)
                        e = t0 + tc
                        o = tb + td
                        zs[0].append(e + o)
                        zs[1].append(e - o)
                        zs[2].append(t0 - tc)
                        zs[3].append(tb - td)
                        t0 = td
                    z0, z2, za, zb = [jnp.concatenate(z, axis=0).astype(bf16) for z in zs]
                    x0 = _dot(t02_ref[0:128, :], z0)
                    x2 = _dot(t02_ref[128:256, :], z2)
                    x1 = _dot(t1_ref[...], jnp.concatenate([za, zb], axis=0))
                    g8 = pl.multiple_of(gi * 8, 8)
                    for k0, xv in ((0, x0), (8, x2), (16, x1)):
                        for kk in range(xv.shape[0] // 16):
                            buf_ref[pl.ds((k0 + kk) * NW + g8, 8), s * D:(s + 1) * D] = _pair(
                                xv[16 * kk:16 * kk + 8], xv[16 * kk + 8:16 * kk + 16])
                return c
            jax.lax.fori_loop(0, NG, fwd, 0, unroll=5)

            @pl.when(b + 1 < B)
            def _():
                x_copy(b + 1).start()

            def mix(k, special):
                if special:
                    w32 = buf_ref[0:NW, :]
                else:
                    w32 = buf_ref[pl.ds(pl.multiple_of(k * NW, 8), NW), :]
                xa = _part(w32, 0)
                xi = _part(w32, 1)
                wc = wf_ref[k, :, 0:D]
                wd = wf_ref[k, :, D:2 * D]
                t1 = _dot(xa, wc)
                t2 = _dot(xi, wd)
                if special:
                    yr, yi = t1, t2
                else:
                    we = (wc.astype(f32) + wd.astype(f32)).astype(bf16)
                    t3 = _dot(xa + xi, we)
                    yr = t1 - t2
                    yi = t3 - (t1 + t2)
                y = jnp.concatenate([yr.reshape(NG, 8, D), yi.reshape(NG, 8, D)], axis=1).reshape(MR, D)
                y_ref[k] = y.astype(bf16)
            mix(0, True)

            def mbody(k, c):
                mix(k, False)
                return c
            jax.lax.fori_loop(1, _NS, mbody, 0, unroll=5)

            def inv(gi):
                m0 = gi * 16 if isinstance(gi, int) else pl.multiple_of(gi * 16, 16)
                y0 = jnp.concatenate([y_ref[kk, pl.ds(m0, 16), :] for kk in range(8)], axis=0)
                y2 = jnp.concatenate([y_ref[8 + kk, pl.ds(m0, 16), :] for kk in range(8)], axis=0)
                y1 = jnp.concatenate([y_ref[16 + kk, pl.ds(m0, 16), :] for kk in range(16)], axis=0)
                z0 = _dot(a02_ref[0:128, :], y0).reshape(8, 16, D)
                z2 = _dot(a02_ref[128:256, :], y2).reshape(8, 16, D)
                ab = _dot(a1_ref[...], y1)
                za = ab[:128].reshape(8, 16, D)
                zb = ab[128:].reshape(8, 16, D)
                e = z0 + z2
                hh = jnp.concatenate([e + za, (z0 - z2) + zb, e - za], axis=1).reshape(GR, D)
                h_store(gi, hh)
                return hh

            def acc(hh, sh, s1, s2):
                d = (hh - sh).reshape(GR // 8, 8, D)
                return s1 + jnp.sum(d, axis=0), s2 + jnp.sum(d * d, axis=0)

            h0 = inv(0)
            sh = jnp.sum(jnp.sum(h0.reshape(GR // 8, 8, D), axis=0), axis=0, keepdims=True) * (1.0 / GR)
            zz = jnp.zeros((8, D), f32)
            s1, s2 = acc(h0, sh, zz, zz)
            s1, s2 = jax.lax.fori_loop(1, NG - 1, lambda gi, c: acc(inv(gi), sh, *c), (s1, s2), unroll=NG - 2)
            hl = inv(NG - 1)
            row = jax.lax.broadcasted_iota(jnp.int32, (GR, D), 0)
            d = jnp.where(row < L - GR * (NG - 1), hl - sh, 0.0).reshape(GR // 8, 8, D)
            s1 = s1 + jnp.sum(d, axis=0)
            s2 = s2 + jnp.sum(d * d, axis=0)
            dm = jnp.sum(s1, axis=0, keepdims=True) * (1.0 / L)
            mu = sh + dm
            var = jnp.maximum(jnp.sum(s2, axis=0, keepdims=True) * (1.0 / L) - dm * dm, 0.0)
            scale = g_ref[...].reshape(1, D).astype(f32) / jnp.sqrt(var + 1e-5)
            shift = b_ref[...].reshape(1, D).astype(f32) - mu * scale
            st_ref[0:1, :] = scale
            st_ref[1:2, :] = shift

        @pl.when(step == 0)
        def _():
            def fin0(gi, c):
                y0 = finish(pltpu.bitcast(buf_ref[h_idx(gi)], f32), 0)
                sh_ref[pl.ds(pl.multiple_of(gi * GR, GR), GR), :] = y0.astype(bf16)
                return c
            jax.lax.fori_loop(0, NG, fin0, 0)

        @pl.when(step >= B)
        def _():
            def fin(j, c):
                gi = (step - B) * GPC + j
                y1 = finish(pltpu.bitcast(buf_ref[h_idx(gi)], f32), 0)
                y0 = sh_ref[pl.ds(pl.multiple_of(gi * GR, GR), GR), :]
                y1b = y1.astype(bf16)
                cols = []
                for jj in range(GR // 16):
                    cols.append(jnp.concatenate(
                        [yy[16 * jj:16 * jj + 16, 128 * cc:128 * (cc + 1)] for yy in (y0, y1b) for cc in range(4)], axis=0))
                sm = jnp.concatenate(cols, axis=1)
                r = _dot(pm_ref[...], sm)
                rr = jnp.concatenate([r[:, 128 * jj:128 * (jj + 1)] for jj in range(GR // 16)], axis=0)
                o_ref[pl.ds(pl.multiple_of(j * 8 * GR, 8 * GR), 8 * GR), :] = rr.astype(bf16)
                return c
            jax.lax.fori_loop(0, GPC, fin, 0, unroll=GPC)

    vm = lambda shape: pl.BlockSpec(shape, lambda s: (0,) * len(shape), pipeline_mode=pl.Buffered(1))
    any_spec = pl.BlockSpec(memory_space=pl.ANY)
    out = pl.pallas_call(
        kernel,
        grid=(B + NCH,),
        in_specs=[any_spec, any_spec, vm((D,)), vm((D,)),
                  vm((256, 128)), vm((256, 256)), vm((256, 128)), vm((256, 256)), vm((512, 128)), vm((128, 128))],
        out_specs=pl.BlockSpec((CH * 8, 128), lambda s: (jnp.maximum(s - B, 0), 0)),
        out_shape=jax.ShapeDtypeStruct((L * 8, 128), x.dtype),
        scratch_shapes=[
            pltpu.VMEM((_NS, 2 * D, 2 * D), bf16),
            pltpu.VMEM((XPAD, D), bf16),
            pltpu.VMEM((_NS * NW, 2 * D), jnp.uint32),
            pltpu.VMEM((_NS, MR, D), bf16),
            pltpu.VMEM((8, D), f32),
            pltpu.VMEM((NG * GR, D), bf16),
            pltpu.SemaphoreType.DMA(()),
            pltpu.SemaphoreType.DMA((NWS,)),
        ],
        compiler_params=pltpu.CompilerParams(
            dimension_semantics=("arbitrary",),
            vmem_limit_bytes=128 * 1024 * 1024,
        ),
    )(x, w, gn_gamma, gn_beta, *_CONSTS)
    return out.reshape(L, 4, B, 128).transpose(2, 0, 1, 3).reshape(B, L, D)
```

```python
import functools
import numpy as np
import jax
import jax.numpy as jnp
import jax.experimental.pallas as pl
import jax.experimental.pallas.tpu as pltpu

_RH = 0.7071067811865476
_C1 = 0.9238795325112867
_C3 = 0.3826834323650898
_N = 64
_HOP = 48
_NS = 32


_MXU_COMPS = [m for m in range(64) if m // 2 >= 8]


def _slot_freqs():
    return ([0] + [4 * k for k in range(1, 8)] + [4 * k + 2 for k in range(8)]
            + [2 * k + 1 for k in range(16)])


def _build_consts():
    n = _N
    th = 2 * np.pi / n
    fr = _slot_freqs()
    p = np.arange(16)

    def fwd_real(k):
        f = fr[k]
        if k == 0:
            return np.stack([np.ones(16), (-1.0) ** p])
        return np.stack([np.cos(th * f * p), -np.sin(th * f * p)])

    t02 = np.zeros((256, 128))
    t1 = np.zeros((256, 256))
    for kk in range(16):
        for cmp in range(2):
            for b in range(8):
                t02[16 * kk + 8 * cmp + b, 16 * b:16 * b + 16] = fwd_real(kk)[cmp]
    for kk in range(16):
        f = fr[16 + kk]
        c = np.cos(th * f * p)
        s = np.sin(th * f * p)
        if f % 4 == 1:
            re, im = (c, -s), (-s, -c)
        else:
            re, im = (c, s), (-s, c)
        for b in range(8):
            for part in range(2):
                c0 = 128 * part + 16 * b
                t1[16 * kk + b, c0:c0 + 16] = re[part]
                t1[16 * kk + 8 + b, c0:c0 + 16] = im[part]
    a02 = np.zeros((256, 128))
    a1 = np.zeros((256, 256))
    for kk in range(8):
        for b in range(8):
            f = fr[kk]
            if kk == 0:
                a02[16 * b:16 * b + 16, b] = 1.0 / n
                a02[16 * b:16 * b + 16, 8 + b] = (-1.0) ** p / n
            else:
                a02[16 * b:16 * b + 16, 16 * kk + b] = 2.0 / n * np.cos(th * f * p)
                a02[16 * b:16 * b + 16, 16 * kk + 8 + b] = -2.0 / n * np.sin(th * f * p)
            f = fr[8 + kk]
            a02[128 + 16 * b:128 + 16 * b + 16, 16 * kk + b] = 2.0 / n * np.cos(th * f * p)
            a02[128 + 16 * b:128 + 16 * b + 16, 16 * kk + 8 + b] = -2.0 / n * np.sin(th * f * p)
    for kk in range(16):
        f = fr[16 + kk]
        c = np.cos(th * f * p)
        s = np.sin(th * f * p)
        sg = -1.0 if f % 4 == 1 else 1.0
        for b in range(8):
            a1[16 * b:16 * b + 16, 16 * kk + b] = 2.0 / n * c
            a1[16 * b:16 * b + 16, 16 * kk + 8 + b] = -2.0 / n * s
            a1[128 + 16 * b:128 + 16 * b + 16, 16 * kk + b] = sg * 2.0 / n * s
            a1[128 + 16 * b:128 + 16 * b + 16, 16 * kk + 8 + b] = sg * 2.0 / n * c
    j = np.arange(16)
    g = np.zeros((64, 16))
    for k in range(32):
        f = fr[k]
        if k == 0:
            g[0] = 1.0
            g[1] = (-1.0) ** j
        else:
            g[2 * k] = np.cos(th * f * j)
            g[2 * k + 1] = np.sin(th * f * j)
    gk = np.zeros((8 * len(_MXU_COMPS), 128))
    for i, m in enumerate(_MXU_COMPS):
        for c in range(8):
            gk[8 * i + c, np.arange(16) * 8 + c] = g[m]
    pm = np.zeros((128, 128))
    for bb in range(2):
        for ct in range(4):
            for l in range(16):
                pm[l * 8 + ct * 2 + bb, (bb * 4 + ct) * 16 + l] = 1.0
    bf = jnp.bfloat16
    return tuple(np.asarray(a, np.float32).astype(bf) for a in (t02, t1, a02, a1, gk, pm))


_CONSTS = _build_consts()


def _gelu(x):
    c = 0.7978845608028654
    hx = 0.5 * x
    return hx + hx * jnp.tanh(x * (c + (c * 0.044715) * (x * x)))


def _pair(lo, hi):
    return pltpu.pack_elementwise([lo, hi], packed_dtype=jnp.bfloat16).astype(jnp.uint32)


def _part(w32, i):
    return pltpu.unpack_elementwise(w32, index=i, packed_dtype=jnp.bfloat16, unpacked_dtype=jnp.float32)


def _dot(a, b):
    return jnp.dot(a, b, preferred_element_type=jnp.float32)


@jax.jit
def pallas_standalone__self_sup_conv_stem_wavlm__speech_kernel(
    x: jax.Array,
    w: jax.Array,
    gn_gamma: jax.Array,
    gn_beta: jax.Array,
):
    B, T, D = x.shape
    K = w.shape[0]
    L = (T - K) // 2 + 1
    assert (T, D, K) == (16000, 512, 31)
    NG = 21
    GR = 8 * _HOP
    XR = 2 * (GR + 16)
    XPAD = 2 * GR * (NG - 1) + XR
    NW = 8 * NG
    MR = 16 * NG
    WC = 64
    NWC = D // WC
    NWS = 5
    GPC = 1
    CH = GPC * GR
    NCH = NG // GPC
    bf16, f32 = jnp.bfloat16, jnp.float32

    def kernel(x_hbm, w_hbm, g_ref, b_ref, t02_ref, t1_ref, a02_ref, a1_ref, gk_ref, pm_ref,
               o_ref, wf_ref, xb_ref, buf_ref, y_ref, st_ref, sh_ref, xsem, wsem):
        step = pl.program_id(0)
        b = jnp.minimum(step, B - 1)

        def x_copy(bb):
            return pltpu.make_async_copy(x_hbm.at[bb], xb_ref.at[pl.ds(0, T)], xsem)

        def x_piece(i):
            n = T // NWC
            return pltpu.make_async_copy(x_hbm.at[0, pl.ds(i * n, n)], xb_ref.at[pl.ds(i * n, n)], xsem)

        def w_copy(ch):
            slot = ch % NWS
            return pltpu.make_async_copy(
                w_hbm.at[:, pl.ds(ch * WC, WC), :], y_ref.at[pl.ds(0, K), pl.ds(slot * WC, WC), :], wsem.at[slot])

        def h_idx(gi):
            if isinstance(gi, int):
                return (pl.ds(GR * (gi // 2), GR), pl.ds(D * (gi % 2), D))
            return (pl.ds(pl.multiple_of((gi // 2) * GR, GR), GR), pl.ds(pl.multiple_of((gi % 2) * D, D), D))

        def h_store(gi, hh):
            buf_ref[h_idx(gi)] = pltpu.bitcast(hh, jnp.uint32)

        def finish(hh, row):
            scale = st_ref[row:row + 1, :]
            shift = st_ref[row + 1:row + 2, :]
            return _gelu(hh * scale + shift)

        @pl.when(step == 0)
        def _():
            for ch in range(2):
                w_copy(ch).start()
            xb_ref[T:XPAD, :] = jnp.zeros((XPAD - T, D), bf16)
            gk = gk_ref[...]

            def wchunk(ch, c):
                w_copy(ch).wait()

                @pl.when(ch + 2 < NWC)
                def _():
                    w_copy(ch + 2).start()
                x_piece(ch).start()
                r0 = pl.multiple_of((ch % NWS) * WC, WC)
                for s in range(2):
                    ntap = 16 if s == 0 else 15

                    def body(ci, c):
                        c0 = pl.multiple_of(ci * 16, 16)
                        vs = [y_ref[2 * j + s, pl.ds(r0 + c0, 16), :].astype(f32) for j in range(ntap)]
                        res = []
                        for hh in range(2):
                            parts = [v[8 * hh:8 * hh + 8] for v in vs]
                            if ntap < 16:
                                parts.append(jnp.zeros((8, D), f32))
                            kt = jnp.concatenate(parts, axis=0).astype(bf16)
                            res.append(_dot(gk, kt))
                        nm = len(_MXU_COMPS)
                        r = jnp.concatenate([res[0].reshape(nm, 8, D), res[1].reshape(nm, 8, D)], axis=1)
                        r = r.astype(bf16)
                        comps = {m: r[i] for i, m in enumerate(_MXU_COMPS)}
                        p = [vs[j] + vs[j + 8] if j + 8 < ntap else vs[j] for j in range(8)]
                        sa, sb, sc, sd = [p[j] + p[j + 4] for j in range(4)]
                        da, db, dc, dd = [p[j] - p[j + 4] for j in range(4)]
                        ev, od = sa + sc, sb + sd
                        ru = (db - dd) * _RH
                        rv = (db + dd) * _RH
                        q = [vs[j] - vs[j + 8] if j + 8 < ntap else vs[j] for j in range(8)]
                        ca, cb, ce = q[1] - q[7], q[3] - q[5], (q[2] - q[6]) * _RH
                        na, nb, ne = q[1] + q[7], q[3] + q[5], (q[2] + q[6]) * _RH
                        c1, c2 = _C1 * ca + _C3 * cb, _C3 * ca - _C1 * cb
                        n1, n2 = _C3 * na + _C1 * nb, _C1 * na - _C3 * nb
                        cp, cm, np_, nm_ = q[0] + ce, q[0] - ce, ne + q[4], ne - q[4]
                        for m, v in ((0, ev + od), (1, ev - od), (8, sa - sc), (9, sb - sd),
                                     (4, da + ru), (5, dc + rv), (12, da - ru), (13, rv - dc),
                                     (2, cp + c1), (3, n1 + np_), (14, cp - c1), (15, n1 - np_),
                                     (6, cm + c2), (7, n2 + nm_), (10, cm - c2), (11, n2 - nm_)):
                            comps[m] = v.astype(bf16)
                        cw = pl.multiple_of(s * D + ch * WC + c0, 16)
                        for m in range(64):
                            wf_ref[m // 2, pl.ds(cw, 16), (m % 2) * D:(m % 2 + 1) * D] = comps[m]
                        return c
                    jax.lax.fori_loop(0, WC // 16, body, 0, unroll=4)
                return c
            jax.lax.fori_loop(0, NWC, wchunk, 0)

        @pl.when(step < B)
        def _():
            @pl.when(step == 0)
            def _():
                for i in range(NWC):
                    x_piece(i).wait()

            @pl.when(step > 0)
            def _():
                x_copy(b).wait()

            def fwd(gi, c):
                r0 = pl.multiple_of(gi * (2 * GR), 2 * GR)
                for s in range(2):
                    def tile(tt):
                        w32 = pltpu.bitcast(xb_ref[pl.ds(r0 + 32 * tt, 32), :], jnp.uint32)
                        return _part(w32, s)
                    zs = [[], [], [], []]
                    t0 = tile(0)
                    for bb in range(8):
                        tb, tc, td = tile(3 * bb + 1), tile(3 * bb + 2), tile(3 * bb + 3)
                        e = t0 + tc
                        o = tb + td
                        zs[0].append(e + o)
                        zs[1].append(e - o)
                        zs[2].append(t0 - tc)
                        zs[3].append(tb - td)
                        t0 = td
                    z0, z2, za, zb = [jnp.concatenate(z, axis=0).astype(bf16) for z in zs]
                    x0 = _dot(t02_ref[0:128, :], z0)
                    x2 = _dot(t02_ref[128:256, :], z2)
                    x1 = _dot(t1_ref[...], jnp.concatenate([za, zb], axis=0))
                    g8 = pl.multiple_of(gi * 8, 8)
                    for k0, xv in ((0, x0), (8, x2), (16, x1)):
                        for kk in range(xv.shape[0] // 16):
                            buf_ref[pl.ds((k0 + kk) * NW + g8, 8), s * D:(s + 1) * D] = _pair(
                                xv[16 * kk:16 * kk + 8], xv[16 * kk + 8:16 * kk + 16])
                return c
            jax.lax.fori_loop(0, NG, fwd, 0, unroll=5)

            @pl.when(b + 1 < B)
            def _():
                x_copy(b + 1).start()

            def mix(k, special):
                if special:
                    w32 = buf_ref[0:NW, :]
                else:
                    w32 = buf_ref[pl.ds(pl.multiple_of(k * NW, 8), NW), :]
                xa = _part(w32, 0)
                xi = _part(w32, 1)
                wc = wf_ref[k, :, 0:D]
                wd = wf_ref[k, :, D:2 * D]
                t1 = _dot(xa, wc)
                t2 = _dot(xi, wd)
                if special:
                    yr, yi = t1, t2
                else:
                    we = (wc.astype(f32) + wd.astype(f32)).astype(bf16)
                    t3 = _dot(xa + xi, we)
                    yr = t1 - t2
                    yi = t3 - (t1 + t2)
                y = jnp.concatenate([yr.reshape(NG, 8, D), yi.reshape(NG, 8, D)], axis=1).reshape(MR, D)
                y_ref[k] = y.astype(bf16)
            mix(0, True)

            def mbody(k, c):
                mix(k, False)
                return c
            jax.lax.fori_loop(1, _NS, mbody, 0, unroll=5)

            def inv(gi):
                m0 = gi * 16 if isinstance(gi, int) else pl.multiple_of(gi * 16, 16)
                y0 = jnp.concatenate([y_ref[kk, pl.ds(m0, 16), :] for kk in range(8)], axis=0)
                y2 = jnp.concatenate([y_ref[8 + kk, pl.ds(m0, 16), :] for kk in range(8)], axis=0)
                y1 = jnp.concatenate([y_ref[16 + kk, pl.ds(m0, 16), :] for kk in range(16)], axis=0)
                z0 = _dot(a02_ref[0:128, :], y0).reshape(8, 16, D)
                z2 = _dot(a02_ref[128:256, :], y2).reshape(8, 16, D)
                ab = _dot(a1_ref[...], y1)
                za = ab[:128].reshape(8, 16, D)
                zb = ab[128:].reshape(8, 16, D)
                e = z0 + z2
                hh = jnp.concatenate([e + za, (z0 - z2) + zb, e - za], axis=1).reshape(GR, D)
                h_store(gi, hh)
                return hh

            def acc(hh, sh, s1, s2):
                d = (hh - sh).reshape(GR // 8, 8, D)
                return s1 + jnp.sum(d, axis=0), s2 + jnp.sum(d * d, axis=0)

            h0 = inv(0)
            sh = jnp.sum(jnp.sum(h0.reshape(GR // 8, 8, D), axis=0), axis=0, keepdims=True) * (1.0 / GR)
            zz = jnp.zeros((8, D), f32)
            s1, s2 = acc(h0, sh, zz, zz)
            s1, s2 = jax.lax.fori_loop(1, NG - 1, lambda gi, c: acc(inv(gi), sh, *c), (s1, s2), unroll=NG - 2)
            hl = inv(NG - 1)
            row = jax.lax.broadcasted_iota(jnp.int32, (GR, D), 0)
            d = jnp.where(row < L - GR * (NG - 1), hl - sh, 0.0).reshape(GR // 8, 8, D)
            s1 = s1 + jnp.sum(d, axis=0)
            s2 = s2 + jnp.sum(d * d, axis=0)
            dm = jnp.sum(s1, axis=0, keepdims=True) * (1.0 / L)
            mu = sh + dm
            var = jnp.maximum(jnp.sum(s2, axis=0, keepdims=True) * (1.0 / L) - dm * dm, 0.0)
            scale = g_ref[...].reshape(1, D).astype(f32) / jnp.sqrt(var + 1e-5)
            shift = b_ref[...].reshape(1, D).astype(f32) - mu * scale
            st_ref[0:1, :] = scale
            st_ref[1:2, :] = shift

        @pl.when(step == 0)
        def _():
            def fin0(gi, c):
                y0 = finish(pltpu.bitcast(buf_ref[h_idx(gi)], f32), 0)
                sh_ref[pl.ds(pl.multiple_of(gi * GR, GR), GR), :] = y0.astype(bf16)
                return c
            jax.lax.fori_loop(0, NG, fin0, 0)

        @pl.when(step >= B)
        def _():
            def fin(j, c):
                gi = (step - B) * GPC + j
                y1 = finish(pltpu.bitcast(buf_ref[h_idx(gi)], f32), 0)
                y0 = sh_ref[pl.ds(pl.multiple_of(gi * GR, GR), GR), :]
                y1b = y1.astype(bf16)
                cols = []
                for jj in range(GR // 16):
                    cols.append(jnp.concatenate(
                        [yy[16 * jj:16 * jj + 16, 128 * cc:128 * (cc + 1)] for yy in (y0, y1b) for cc in range(4)], axis=0))
                sm = jnp.concatenate(cols, axis=1)
                r = _dot(pm_ref[...], sm)
                rr = jnp.concatenate([r[:, 128 * jj:128 * (jj + 1)] for jj in range(GR // 16)], axis=0)
                o_ref[pl.ds(pl.multiple_of(j * 8 * GR, 8 * GR), 8 * GR), :] = rr.astype(bf16)
                return c
            jax.lax.fori_loop(0, GPC, fin, 0, unroll=GPC)

    vm = lambda shape: pl.BlockSpec(shape, lambda s: (0,) * len(shape), pipeline_mode=pl.Buffered(1))
    any_spec = pl.BlockSpec(memory_space=pl.ANY)
    out = pl.pallas_call(
        kernel,
        grid=(B + NCH,),
        in_specs=[any_spec, any_spec, vm((D,)), vm((D,)),
                  vm((256, 128)), vm((256, 256)), vm((256, 128)), vm((256, 256)), vm((8 * len(_MXU_COMPS), 128)), vm((128, 128))],
        out_specs=pl.BlockSpec((CH * 8, 128), lambda s: (jnp.maximum(s - B, 0), 0)),
        out_shape=jax.ShapeDtypeStruct((L * 8, 128), x.dtype),
        scratch_shapes=[
            pltpu.VMEM((_NS, 2 * D, 2 * D), bf16),
            pltpu.VMEM((XPAD, D), bf16),
            pltpu.VMEM((_NS * NW, 2 * D), jnp.uint32),
            pltpu.VMEM((_NS, MR, D), bf16),
            pltpu.VMEM((8, D), f32),
            pltpu.VMEM((NG * GR, D), bf16),
            pltpu.SemaphoreType.DMA(()),
            pltpu.SemaphoreType.DMA((NWS,)),
        ],
        compiler_params=pltpu.CompilerParams(
            dimension_semantics=("arbitrary",),
            vmem_limit_bytes=128 * 1024 * 1024,
        ),
    )(x, w, gn_gamma, gn_beta, *_CONSTS)
    return out.reshape(L, 4, B, 128).transpose(2, 0, 1, 3).reshape(B, L, D)
```

```python
import functools
import numpy as np
import jax
import jax.numpy as jnp
import jax.experimental.pallas as pl
import jax.experimental.pallas.tpu as pltpu

_RH = 0.7071067811865476
_C1 = 0.9238795325112867
_C3 = 0.3826834323650898
_N = 64
_HOP = 48
_NS = 32


_MXU_COMPS = [m for m in range(64) if m // 2 >= 8]


def _slot_freqs():
    return ([0] + [4 * k for k in range(1, 8)] + [4 * k + 2 for k in range(8)]
            + [2 * k + 1 for k in range(16)])


def _build_consts():
    n = _N
    th = 2 * np.pi / n
    fr = _slot_freqs()
    p = np.arange(16)

    def fwd_real(k):
        f = fr[k]
        if k == 0:
            return np.stack([np.ones(16), (-1.0) ** p])
        return np.stack([np.cos(th * f * p), -np.sin(th * f * p)])

    t02 = np.zeros((256, 128))
    t1 = np.zeros((256, 256))
    for kk in range(16):
        for cmp in range(2):
            for b in range(8):
                t02[16 * kk + 8 * cmp + b, 16 * b:16 * b + 16] = fwd_real(kk)[cmp]
    for kk in range(16):
        f = fr[16 + kk]
        c = np.cos(th * f * p)
        s = np.sin(th * f * p)
        if f % 4 == 1:
            re, im = (c, -s), (-s, -c)
        else:
            re, im = (c, s), (-s, c)
        for b in range(8):
            for part in range(2):
                c0 = 128 * part + 16 * b
                t1[16 * kk + b, c0:c0 + 16] = re[part]
                t1[16 * kk + 8 + b, c0:c0 + 16] = im[part]
    a02 = np.zeros((256, 128))
    a1 = np.zeros((256, 256))
    for kk in range(8):
        for b in range(8):
            f = fr[kk]
            if kk == 0:
                a02[16 * b:16 * b + 16, b] = 1.0 / n
                a02[16 * b:16 * b + 16, 8 + b] = (-1.0) ** p / n
            else:
                a02[16 * b:16 * b + 16, 16 * kk + b] = 2.0 / n * np.cos(th * f * p)
                a02[16 * b:16 * b + 16, 16 * kk + 8 + b] = -2.0 / n * np.sin(th * f * p)
            f = fr[8 + kk]
            a02[128 + 16 * b:128 + 16 * b + 16, 16 * kk + b] = 2.0 / n * np.cos(th * f * p)
            a02[128 + 16 * b:128 + 16 * b + 16, 16 * kk + 8 + b] = -2.0 / n * np.sin(th * f * p)
    for kk in range(16):
        f = fr[16 + kk]
        c = np.cos(th * f * p)
        s = np.sin(th * f * p)
        sg = -1.0 if f % 4 == 1 else 1.0
        for b in range(8):
            a1[16 * b:16 * b + 16, 16 * kk + b] = 2.0 / n * c
            a1[16 * b:16 * b + 16, 16 * kk + 8 + b] = -2.0 / n * s
            a1[128 + 16 * b:128 + 16 * b + 16, 16 * kk + b] = sg * 2.0 / n * s
            a1[128 + 16 * b:128 + 16 * b + 16, 16 * kk + 8 + b] = sg * 2.0 / n * c
    j = np.arange(16)
    g = np.zeros((64, 16))
    for k in range(32):
        f = fr[k]
        if k == 0:
            g[0] = 1.0
            g[1] = (-1.0) ** j
        else:
            g[2 * k] = np.cos(th * f * j)
            g[2 * k + 1] = np.sin(th * f * j)
    gk = np.zeros((8 * len(_MXU_COMPS), 128))
    for i, m in enumerate(_MXU_COMPS):
        for c in range(8):
            gk[8 * i + c, np.arange(16) * 8 + c] = g[m]
    pm = np.zeros((128, 128))
    for bb in range(2):
        for ct in range(4):
            for l in range(16):
                pm[l * 8 + ct * 2 + bb, (bb * 4 + ct) * 16 + l] = 1.0
    bf = jnp.bfloat16
    return tuple(np.asarray(a, np.float32).astype(bf) for a in (t02, t1, a02, a1, gk, pm))


_CONSTS = _build_consts()


def _gelu(x):
    c = 0.7978845608028654
    hx = 0.5 * x
    return hx + hx * jnp.tanh(x * (c + (c * 0.044715) * (x * x)))


def _pair(lo, hi):
    return pltpu.pack_elementwise([lo, hi], packed_dtype=jnp.bfloat16).astype(jnp.uint32)


def _part(w32, i):
    return pltpu.unpack_elementwise(w32, index=i, packed_dtype=jnp.bfloat16, unpacked_dtype=jnp.float32)


def _dot(a, b):
    return jnp.dot(a, b, preferred_element_type=jnp.float32)


@jax.jit
def pallas_standalone__self_sup_conv_stem_wavlm__speech_kernel(
    x: jax.Array,
    w: jax.Array,
    gn_gamma: jax.Array,
    gn_beta: jax.Array,
):
    B, T, D = x.shape
    K = w.shape[0]
    L = (T - K) // 2 + 1
    assert (T, D, K) == (16000, 512, 31)
    NG = 21
    GR = 8 * _HOP
    XR = 2 * (GR + 16)
    XPAD = 2 * GR * (NG - 1) + XR
    NW = 8 * NG
    MR = 16 * NG
    WC = 64
    NWC = D // WC
    NWS = 5
    GPC = 1
    CH = GPC * GR
    NCH = NG // GPC
    bf16, f32 = jnp.bfloat16, jnp.float32

    def kernel(x_hbm, w_hbm, g_ref, b_ref, t02_ref, t1_ref, a02_ref, a1_ref, gk_ref, pm_ref,
               o_ref, wf_ref, xb_ref, buf_ref, y_ref, st_ref, sh_ref, xsem, wsem):
        step = pl.program_id(0)
        b = jnp.minimum(step, B - 1)

        def x_copy(bb):
            return pltpu.make_async_copy(x_hbm.at[bb], xb_ref.at[pl.ds(0, T)], xsem.at[0])

        def x_piece(i):
            n = T // NWC
            return pltpu.make_async_copy(x_hbm.at[0, pl.ds(i * n, n)], xb_ref.at[pl.ds(i * n, n)], xsem.at[i // 3])

        def w_copy(ch):
            slot = ch % NWS
            return pltpu.make_async_copy(
                w_hbm.at[:, pl.ds(ch * WC, WC), :], y_ref.at[pl.ds(0, K), pl.ds(slot * WC, WC), :], wsem.at[slot])

        def h_idx(gi):
            if isinstance(gi, int):
                return (pl.ds(GR * (gi // 2), GR), pl.ds(D * (gi % 2), D))
            return (pl.ds(pl.multiple_of((gi // 2) * GR, GR), GR), pl.ds(pl.multiple_of((gi % 2) * D, D), D))

        def h_store(gi, hh):
            buf_ref[h_idx(gi)] = pltpu.bitcast(hh, jnp.uint32)

        def finish(hh, row):
            scale = st_ref[row:row + 1, :]
            shift = st_ref[row + 1:row + 2, :]
            return _gelu(hh * scale + shift)

        @pl.when(step == 0)
        def _():
            for ch in range(2):
                w_copy(ch).start()
            xb_ref[T:XPAD, :] = jnp.zeros((XPAD - T, D), bf16)
            gk = gk_ref[...]

            def wchunk(ch, c):
                w_copy(ch).wait()

                @pl.when(ch + 2 < NWC)
                def _():
                    w_copy(ch + 2).start()
                x_piece(ch).start()
                r0 = pl.multiple_of((ch % NWS) * WC, WC)
                for s in range(2):
                    ntap = 16 if s == 0 else 15

                    def body(ci, c):
                        c0 = pl.multiple_of(ci * 16, 16)
                        vs = [y_ref[2 * j + s, pl.ds(r0 + c0, 16), :].astype(f32) for j in range(ntap)]
                        res = []
                        for hh in range(2):
                            parts = [v[8 * hh:8 * hh + 8] for v in vs]
                            if ntap < 16:
                                parts.append(jnp.zeros((8, D), f32))
                            kt = jnp.concatenate(parts, axis=0).astype(bf16)
                            res.append(_dot(gk, kt))
                        nm = len(_MXU_COMPS)
                        r = jnp.concatenate([res[0].reshape(nm, 8, D), res[1].reshape(nm, 8, D)], axis=1)
                        r = r.astype(bf16)
                        comps = {m: r[i] for i, m in enumerate(_MXU_COMPS)}
                        p = [vs[j] + vs[j + 8] if j + 8 < ntap else vs[j] for j in range(8)]
                        sa, sb, sc, sd = [p[j] + p[j + 4] for j in range(4)]
                        da, db, dc, dd = [p[j] - p[j + 4] for j in range(4)]
                        ev, od = sa + sc, sb + sd
                        ru = (db - dd) * _RH
                        rv = (db + dd) * _RH
                        q = [vs[j] - vs[j + 8] if j + 8 < ntap else vs[j] for j in range(8)]
                        ca, cb, ce = q[1] - q[7], q[3] - q[5], (q[2] - q[6]) * _RH
                        na, nb, ne = q[1] + q[7], q[3] + q[5], (q[2] + q[6]) * _RH
                        c1, c2 = _C1 * ca + _C3 * cb, _C3 * ca - _C1 * cb
                        n1, n2 = _C3 * na + _C1 * nb, _C1 * na - _C3 * nb
                        cp, cm, np_, nm_ = q[0] + ce, q[0] - ce, ne + q[4], ne - q[4]
                        for m, v in ((0, ev + od), (1, ev - od), (8, sa - sc), (9, sb - sd),
                                     (4, da + ru), (5, dc + rv), (12, da - ru), (13, rv - dc),
                                     (2, cp + c1), (3, n1 + np_), (14, cp - c1), (15, n1 - np_),
                                     (6, cm + c2), (7, n2 + nm_), (10, cm - c2), (11, n2 - nm_)):
                            comps[m] = v.astype(bf16)
                        cw = pl.multiple_of(s * D + ch * WC + c0, 16)
                        for m in range(64):
                            wf_ref[m // 2, pl.ds(cw, 16), (m % 2) * D:(m % 2 + 1) * D] = comps[m]
                        return c
                    jax.lax.fori_loop(0, WC // 16, body, 0, unroll=4)
                return c
            jax.lax.fori_loop(0, NWC, wchunk, 0)

        @pl.when(step < B)
        def _():
            @pl.when(step > 0)
            def _():
                x_copy(b).wait()

            def fwd(gi, c):
                r0 = pl.multiple_of(gi * (2 * GR), 2 * GR)
                for s in range(2):
                    def tile(tt):
                        w32 = pltpu.bitcast(xb_ref[pl.ds(r0 + 32 * tt, 32), :], jnp.uint32)
                        return _part(w32, s)
                    zs = [[], [], [], []]
                    t0 = tile(0)
                    for bb in range(8):
                        tb, tc, td = tile(3 * bb + 1), tile(3 * bb + 2), tile(3 * bb + 3)
                        e = t0 + tc
                        o = tb + td
                        zs[0].append(e + o)
                        zs[1].append(e - o)
                        zs[2].append(t0 - tc)
                        zs[3].append(tb - td)
                        t0 = td
                    z0, z2, za, zb = [jnp.concatenate(z, axis=0).astype(bf16) for z in zs]
                    x0 = _dot(t02_ref[0:128, :], z0)
                    x2 = _dot(t02_ref[128:256, :], z2)
                    x1 = _dot(t1_ref[...], jnp.concatenate([za, zb], axis=0))
                    g8 = pl.multiple_of(gi * 8, 8)
                    for k0, xv in ((0, x0), (8, x2), (16, x1)):
                        for kk in range(xv.shape[0] // 16):
                            buf_ref[pl.ds((k0 + kk) * NW + g8, 8), s * D:(s + 1) * D] = _pair(
                                xv[16 * kk:16 * kk + 8], xv[16 * kk + 8:16 * kk + 16])
                return c

            def fpart(p, c):
                for pp in range(3):
                    @pl.when(jnp.logical_and(step == 0, p == pp))
                    def _():
                        for i in range(3 * pp, min(3 * pp + 3, NWC)):
                            x_piece(i).wait()
                jax.lax.fori_loop(0, NG // 3, lambda j, c2: fwd(p * (NG // 3) + j, c2), 0, unroll=NG // 3)
                return c
            jax.lax.fori_loop(0, 3, fpart, 0)

            @pl.when(b + 1 < B)
            def _():
                x_copy(b + 1).start()

            def mix(k, special):
                if special:
                    w32 = buf_ref[0:NW, :]
                else:
                    w32 = buf_ref[pl.ds(pl.multiple_of(k * NW, 8), NW), :]
                xa = _part(w32, 0)
                xi = _part(w32, 1)
                wc = wf_ref[k, :, 0:D]
                wd = wf_ref[k, :, D:2 * D]
                t1 = _dot(xa, wc)
                t2 = _dot(xi, wd)
                if special:
                    yr, yi = t1, t2
                else:
                    we = (wc.astype(f32) + wd.astype(f32)).astype(bf16)
                    t3 = _dot(xa + xi, we)
                    yr = t1 - t2
                    yi = t3 - (t1 + t2)
                y = jnp.concatenate([yr.reshape(NG, 8, D), yi.reshape(NG, 8, D)], axis=1).reshape(MR, D)
                y_ref[k] = y.astype(bf16)
            mix(0, True)

            def mbody(k, c):
                mix(k, False)
                return c
            jax.lax.fori_loop(1, _NS, mbody, 0, unroll=5)

            def inv(gi):
                m0 = gi * 16 if isinstance(gi, int) else pl.multiple_of(gi * 16, 16)
                y0 = jnp.concatenate([y_ref[kk, pl.ds(m0, 16), :] for kk in range(8)], axis=0)
                y2 = jnp.concatenate([y_ref[8 + kk, pl.ds(m0, 16), :] for kk in range(8)], axis=0)
                y1 = jnp.concatenate([y_ref[16 + kk, pl.ds(m0, 16), :] for kk in range(16)], axis=0)
                z0 = _dot(a02_ref[0:128, :], y0).reshape(8, 16, D)
                z2 = _dot(a02_ref[128:256, :], y2).reshape(8, 16, D)
                ab = _dot(a1_ref[...], y1)
                za = ab[:128].reshape(8, 16, D)
                zb = ab[128:].reshape(8, 16, D)
                e = z0 + z2
                hh = jnp.concatenate([e + za, (z0 - z2) + zb, e - za], axis=1).reshape(GR, D)
                h_store(gi, hh)
                return hh

            def acc(hh, sh, s1, s2):
                d = (hh - sh).reshape(GR // 8, 8, D)
                return s1 + jnp.sum(d, axis=0), s2 + jnp.sum(d * d, axis=0)

            h0 = inv(0)
            sh = jnp.sum(jnp.sum(h0.reshape(GR // 8, 8, D), axis=0), axis=0, keepdims=True) * (1.0 / GR)
            zz = jnp.zeros((8, D), f32)
            s1, s2 = acc(h0, sh, zz, zz)
            s1, s2 = jax.lax.fori_loop(1, NG - 1, lambda gi, c: acc(inv(gi), sh, *c), (s1, s2), unroll=NG - 2)
            hl = inv(NG - 1)
            row = jax.lax.broadcasted_iota(jnp.int32, (GR, D), 0)
            d = jnp.where(row < L - GR * (NG - 1), hl - sh, 0.0).reshape(GR // 8, 8, D)
            s1 = s1 + jnp.sum(d, axis=0)
            s2 = s2 + jnp.sum(d * d, axis=0)
            dm = jnp.sum(s1, axis=0, keepdims=True) * (1.0 / L)
            mu = sh + dm
            var = jnp.maximum(jnp.sum(s2, axis=0, keepdims=True) * (1.0 / L) - dm * dm, 0.0)
            scale = g_ref[...].reshape(1, D).astype(f32) / jnp.sqrt(var + 1e-5)
            shift = b_ref[...].reshape(1, D).astype(f32) - mu * scale
            st_ref[0:1, :] = scale
            st_ref[1:2, :] = shift

        @pl.when(step == 0)
        def _():
            def fin0(gi, c):
                y0 = finish(pltpu.bitcast(buf_ref[h_idx(gi)], f32), 0)
                sh_ref[pl.ds(pl.multiple_of(gi * GR, GR), GR), :] = y0.astype(bf16)
                return c
            jax.lax.fori_loop(0, NG, fin0, 0)

        @pl.when(step >= B)
        def _():
            def fin(j, c):
                gi = (step - B) * GPC + j
                y1 = finish(pltpu.bitcast(buf_ref[h_idx(gi)], f32), 0)
                y0 = sh_ref[pl.ds(pl.multiple_of(gi * GR, GR), GR), :]
                y1b = y1.astype(bf16)
                cols = []
                for jj in range(GR // 16):
                    cols.append(jnp.concatenate(
                        [yy[16 * jj:16 * jj + 16, 128 * cc:128 * (cc + 1)] for yy in (y0, y1b) for cc in range(4)], axis=0))
                sm = jnp.concatenate(cols, axis=1)
                r = _dot(pm_ref[...], sm)
                rr = jnp.concatenate([r[:, 128 * jj:128 * (jj + 1)] for jj in range(GR // 16)], axis=0)
                o_ref[pl.ds(pl.multiple_of(j * 8 * GR, 8 * GR), 8 * GR), :] = rr.astype(bf16)
                return c
            jax.lax.fori_loop(0, GPC, fin, 0, unroll=GPC)

    vm = lambda shape: pl.BlockSpec(shape, lambda s: (0,) * len(shape), pipeline_mode=pl.Buffered(1))
    any_spec = pl.BlockSpec(memory_space=pl.ANY)
    out = pl.pallas_call(
        kernel,
        grid=(B + NCH,),
        in_specs=[any_spec, any_spec, vm((D,)), vm((D,)),
                  vm((256, 128)), vm((256, 256)), vm((256, 128)), vm((256, 256)), vm((8 * len(_MXU_COMPS), 128)), vm((128, 128))],
        out_specs=pl.BlockSpec((CH * 8, 128), lambda s: (jnp.maximum(s - B, 0), 0)),
        out_shape=jax.ShapeDtypeStruct((L * 8, 128), x.dtype),
        scratch_shapes=[
            pltpu.VMEM((_NS, 2 * D, 2 * D), bf16),
            pltpu.VMEM((XPAD, D), bf16),
            pltpu.VMEM((_NS * NW, 2 * D), jnp.uint32),
            pltpu.VMEM((_NS, MR, D), bf16),
            pltpu.VMEM((8, D), f32),
            pltpu.VMEM((NG * GR, D), bf16),
            pltpu.SemaphoreType.DMA((3,)),
            pltpu.SemaphoreType.DMA((NWS,)),
        ],
        compiler_params=pltpu.CompilerParams(
            dimension_semantics=("arbitrary",),
            vmem_limit_bytes=128 * 1024 * 1024,
        ),
    )(x, w, gn_gamma, gn_beta, *_CONSTS)
    return out.reshape(L, 4, B, 128).transpose(2, 0, 1, 3).reshape(B, L, D)
```

```python
import numpy as np
import jax
import jax.numpy as jnp
import jax.experimental.pallas as pl
import jax.experimental.pallas.tpu as pltpu

_RH = 0.7071067811865476
_C1 = 0.9238795325112867
_C3 = 0.3826834323650898
_N = 64
_HOP = 48
_NS = 32


_MXU_COMPS = [m for m in range(64) if m // 2 >= 8]


def _slot_freqs():
    return ([0] + [4 * k for k in range(1, 8)] + [4 * k + 2 for k in range(8)]
            + [2 * k + 1 for k in range(16)])


def _build_consts():
    n = _N
    th = 2 * np.pi / n
    fr = _slot_freqs()
    p = np.arange(16)

    def fwd_real(k):
        f = fr[k]
        if k == 0:
            return np.stack([np.ones(16), (-1.0) ** p])
        return np.stack([np.cos(th * f * p), -np.sin(th * f * p)])

    t02 = np.zeros((256, 128))
    t1 = np.zeros((256, 256))
    for kk in range(16):
        for cmp in range(2):
            for b in range(8):
                t02[16 * kk + 8 * cmp + b, 16 * b:16 * b + 16] = fwd_real(kk)[cmp]
    for kk in range(16):
        f = fr[16 + kk]
        c = np.cos(th * f * p)
        s = np.sin(th * f * p)
        if f % 4 == 1:
            re, im = (c, -s), (-s, -c)
        else:
            re, im = (c, s), (-s, c)
        for b in range(8):
            for part in range(2):
                c0 = 128 * part + 16 * b
                t1[16 * kk + b, c0:c0 + 16] = re[part]
                t1[16 * kk + 8 + b, c0:c0 + 16] = im[part]
    a02 = np.zeros((256, 128))
    a1 = np.zeros((256, 256))
    for kk in range(8):
        for b in range(8):
            f = fr[kk]
            if kk == 0:
                a02[16 * b:16 * b + 16, b] = 1.0 / n
                a02[16 * b:16 * b + 16, 8 + b] = (-1.0) ** p / n
            else:
                a02[16 * b:16 * b + 16, 16 * kk + b] = 2.0 / n * np.cos(th * f * p)
                a02[16 * b:16 * b + 16, 16 * kk + 8 + b] = -2.0 / n * np.sin(th * f * p)
            f = fr[8 + kk]
            a02[128 + 16 * b:128 + 16 * b + 16, 16 * kk + b] = 2.0 / n * np.cos(th * f * p)
            a02[128 + 16 * b:128 + 16 * b + 16, 16 * kk + 8 + b] = -2.0 / n * np.sin(th * f * p)
    for kk in range(16):
        f = fr[16 + kk]
        c = np.cos(th * f * p)
        s = np.sin(th * f * p)
        sg = -1.0 if f % 4 == 1 else 1.0
        for b in range(8):
            a1[16 * b:16 * b + 16, 16 * kk + b] = 2.0 / n * c
            a1[16 * b:16 * b + 16, 16 * kk + 8 + b] = -2.0 / n * s
            a1[128 + 16 * b:128 + 16 * b + 16, 16 * kk + b] = sg * 2.0 / n * s
            a1[128 + 16 * b:128 + 16 * b + 16, 16 * kk + 8 + b] = sg * 2.0 / n * c
    j = np.arange(16)
    g = np.zeros((64, 16))
    for k in range(32):
        f = fr[k]
        if k == 0:
            g[0] = 1.0
            g[1] = (-1.0) ** j
        else:
            g[2 * k] = np.cos(th * f * j)
            g[2 * k + 1] = np.sin(th * f * j)
    gk = np.zeros((8 * len(_MXU_COMPS), 128))
    for i, m in enumerate(_MXU_COMPS):
        for c in range(8):
            gk[8 * i + c, np.arange(16) * 8 + c] = g[m]
    pm = np.zeros((128, 128))
    for bb in range(2):
        for ct in range(4):
            for l in range(16):
                pm[l * 8 + ct * 2 + bb, (bb * 4 + ct) * 16 + l] = 1.0
    bf = jnp.bfloat16
    return tuple(np.asarray(a, np.float32).astype(bf) for a in (t02, t1, a02, a1, gk, pm))


_CONSTS = _build_consts()


def _gelu(x):
    c = 0.7978845608028654
    hx = 0.5 * x
    return hx + hx * jnp.tanh(x * (c + (c * 0.044715) * (x * x)))


def _pair(lo, hi):
    return pltpu.pack_elementwise([lo, hi], packed_dtype=jnp.bfloat16).astype(jnp.uint32)


def _part(w32, i):
    return pltpu.unpack_elementwise(w32, index=i, packed_dtype=jnp.bfloat16, unpacked_dtype=jnp.float32)


def _dot(a, b):
    return jnp.dot(a, b, preferred_element_type=jnp.float32)


@jax.jit
def pallas_standalone__self_sup_conv_stem_wavlm__speech_kernel(
    x: jax.Array,
    w: jax.Array,
    gn_gamma: jax.Array,
    gn_beta: jax.Array,
):
    B, T, D = x.shape
    K = w.shape[0]
    L = (T - K) // 2 + 1
    assert (T, D, K) == (16000, 512, 31)
    NG = 21
    GR = 8 * _HOP
    XR = 2 * (GR + 16)
    XPAD = 2 * GR * (NG - 1) + XR
    NW = 8 * NG
    MR = 16 * NG
    WC = 64
    NWC = D // WC
    NWS = 5
    GPC = 1
    CH = GPC * GR
    NCH = NG // GPC
    bf16, f32 = jnp.bfloat16, jnp.float32

    def kernel(x_hbm, w_hbm, g_ref, b_ref, t02_ref, t1_ref, a02_ref, a1_ref, gk_ref, pm_ref,
               o_ref, wf_ref, xb_ref, buf_ref, y_ref, st_ref, sh_ref, xsem, wsem):
        step = pl.program_id(0)
        b = jnp.minimum(step, B - 1)

        def x_copy(bb):
            return pltpu.make_async_copy(x_hbm.at[bb], xb_ref.at[pl.ds(0, T)], xsem.at[0])

        def x_piece(i):
            n = T // NWC
            return pltpu.make_async_copy(x_hbm.at[0, pl.ds(i * n, n)], xb_ref.at[pl.ds(i * n, n)], xsem.at[i // 3])

        def w_copy(ch):
            slot = ch % NWS
            return pltpu.make_async_copy(
                w_hbm.at[:, pl.ds(ch * WC, WC), :], y_ref.at[pl.ds(0, K), pl.ds(slot * WC, WC), :], wsem.at[slot])

        def h_idx(gi):
            if isinstance(gi, int):
                return (pl.ds(GR * (gi // 2), GR), pl.ds(D * (gi % 2), D))
            return (pl.ds(pl.multiple_of((gi // 2) * GR, GR), GR), pl.ds(pl.multiple_of((gi % 2) * D, D), D))

        def h_store(gi, hh):
            buf_ref[h_idx(gi)] = pltpu.bitcast(hh, jnp.uint32)

        def finish(hh, row):
            scale = st_ref[row:row + 1, :]
            shift = st_ref[row + 1:row + 2, :]
            return _gelu(hh * scale + shift)

        @pl.when(step == 0)
        def _():
            for ch in range(3):
                w_copy(ch).start()
            xb_ref[T:XPAD, :] = jnp.zeros((XPAD - T, D), bf16)
            gk = gk_ref[...]

            def wchunk(ch, c):
                w_copy(ch).wait()

                @pl.when(ch + 3 < NWC)
                def _():
                    w_copy(ch + 3).start()
                x_piece(ch).start()
                r0 = pl.multiple_of((ch % NWS) * WC, WC)
                for s in range(2):
                    ntap = 16 if s == 0 else 15

                    def body(ci, c):
                        c0 = pl.multiple_of(ci * 16, 16)
                        vs = [y_ref[2 * j + s, pl.ds(r0 + c0, 16), :].astype(f32) for j in range(ntap)]
                        res = []
                        for hh in range(2):
                            parts = [v[8 * hh:8 * hh + 8] for v in vs]
                            if ntap < 16:
                                parts.append(jnp.zeros((8, D), f32))
                            kt = jnp.concatenate(parts, axis=0).astype(bf16)
                            res.append(_dot(gk, kt))
                        nm = len(_MXU_COMPS)
                        r = jnp.concatenate([res[0].reshape(nm, 8, D), res[1].reshape(nm, 8, D)], axis=1)
                        r = r.astype(bf16)
                        comps = {m: r[i] for i, m in enumerate(_MXU_COMPS)}
                        p = [vs[j] + vs[j + 8] if j + 8 < ntap else vs[j] for j in range(8)]
                        sa, sb, sc, sd = [p[j] + p[j + 4] for j in range(4)]
                        da, db, dc, dd = [p[j] - p[j + 4] for j in range(4)]
                        ev, od = sa + sc, sb + sd
                        ru = (db - dd) * _RH
                        rv = (db + dd) * _RH
                        q = [vs[j] - vs[j + 8] if j + 8 < ntap else vs[j] for j in range(8)]
                        ca, cb, ce = q[1] - q[7], q[3] - q[5], (q[2] - q[6]) * _RH
                        na, nb, ne = q[1] + q[7], q[3] + q[5], (q[2] + q[6]) * _RH
                        c1, c2 = _C1 * ca + _C3 * cb, _C3 * ca - _C1 * cb
                        n1, n2 = _C3 * na + _C1 * nb, _C1 * na - _C3 * nb
                        cp, cm, np_, nm_ = q[0] + ce, q[0] - ce, ne + q[4], ne - q[4]
                        for m, v in ((0, ev + od), (1, ev - od), (8, sa - sc), (9, sb - sd),
                                     (4, da + ru), (5, dc + rv), (12, da - ru), (13, rv - dc),
                                     (2, cp + c1), (3, n1 + np_), (14, cp - c1), (15, n1 - np_),
                                     (6, cm + c2), (7, n2 + nm_), (10, cm - c2), (11, n2 - nm_)):
                            comps[m] = v.astype(bf16)
                        cw = pl.multiple_of(s * D + ch * WC + c0, 16)
                        for m in range(64):
                            wf_ref[m // 2, pl.ds(cw, 16), (m % 2) * D:(m % 2 + 1) * D] = comps[m]
                        return c
                    jax.lax.fori_loop(0, WC // 16, body, 0, unroll=4)
                return c
            jax.lax.fori_loop(0, NWC, wchunk, 0)

        @pl.when(step < B)
        def _():
            @pl.when(step > 0)
            def _():
                x_copy(b).wait()

            def fwd(gi, c):
                r0 = pl.multiple_of(gi * (2 * GR), 2 * GR)
                for s in range(2):
                    def tile(tt):
                        w32 = pltpu.bitcast(xb_ref[pl.ds(r0 + 32 * tt, 32), :], jnp.uint32)
                        return _part(w32, s)
                    zs = [[], [], [], []]
                    t0 = tile(0)
                    for bb in range(8):
                        tb, tc, td = tile(3 * bb + 1), tile(3 * bb + 2), tile(3 * bb + 3)
                        e = t0 + tc
                        o = tb + td
                        zs[0].append(e + o)
                        zs[1].append(e - o)
                        zs[2].append(t0 - tc)
                        zs[3].append(tb - td)
                        t0 = td
                    z0, z2, za, zb = [jnp.concatenate(z, axis=0).astype(bf16) for z in zs]
                    x0 = _dot(t02_ref[0:128, :], z0)
                    x2 = _dot(t02_ref[128:256, :], z2)
                    x1 = _dot(t1_ref[...], jnp.concatenate([za, zb], axis=0))
                    g8 = pl.multiple_of(gi * 8, 8)
                    for k0, xv in ((0, x0), (8, x2), (16, x1)):
                        for kk in range(xv.shape[0] // 16):
                            buf_ref[pl.ds((k0 + kk) * NW + g8, 8), s * D:(s + 1) * D] = _pair(
                                xv[16 * kk:16 * kk + 8], xv[16 * kk + 8:16 * kk + 16])
                return c

            def fpart(p, c):
                for pp in range(3):
                    @pl.when(jnp.logical_and(step == 0, p == pp))
                    def _():
                        for i in range(3 * pp, min(3 * pp + 3, NWC)):
                            x_piece(i).wait()
                jax.lax.fori_loop(0, NG // 3, lambda j, c2: fwd(p * (NG // 3) + j, c2), 0, unroll=NG // 3)
                return c
            jax.lax.fori_loop(0, 3, fpart, 0)

            @pl.when(b + 1 < B)
            def _():
                x_copy(b + 1).start()

            def mix(k, special):
                if special:
                    w32 = buf_ref[0:NW, :]
                else:
                    w32 = buf_ref[pl.ds(pl.multiple_of(k * NW, 8), NW), :]
                xa = _part(w32, 0)
                xi = _part(w32, 1)
                wc = wf_ref[k, :, 0:D]
                wd = wf_ref[k, :, D:2 * D]
                t1 = _dot(xa, wc)
                t2 = _dot(xi, wd)
                if special:
                    yr, yi = t1, t2
                else:
                    we = (wc.astype(f32) + wd.astype(f32)).astype(bf16)
                    t3 = _dot(xa + xi, we)
                    yr = t1 - t2
                    yi = t3 - (t1 + t2)
                y = jnp.concatenate([yr.reshape(NG, 8, D), yi.reshape(NG, 8, D)], axis=1).reshape(MR, D)
                y_ref[k] = y.astype(bf16)
            mix(0, True)

            def mbody(k, c):
                mix(k, False)
                return c
            jax.lax.fori_loop(1, _NS, mbody, 0, unroll=5)

            def inv(gi):
                m0 = gi * 16 if isinstance(gi, int) else pl.multiple_of(gi * 16, 16)
                y0 = jnp.concatenate([y_ref[kk, pl.ds(m0, 16), :] for kk in range(8)], axis=0)
                y2 = jnp.concatenate([y_ref[8 + kk, pl.ds(m0, 16), :] for kk in range(8)], axis=0)
                y1 = jnp.concatenate([y_ref[16 + kk, pl.ds(m0, 16), :] for kk in range(16)], axis=0)
                z0 = _dot(a02_ref[0:128, :], y0).reshape(8, 16, D)
                z2 = _dot(a02_ref[128:256, :], y2).reshape(8, 16, D)
                ab = _dot(a1_ref[...], y1)
                za = ab[:128].reshape(8, 16, D)
                zb = ab[128:].reshape(8, 16, D)
                e = z0 + z2
                hh = jnp.concatenate([e + za, (z0 - z2) + zb, e - za], axis=1).reshape(GR, D)
                h_store(gi, hh)
                return hh

            def acc(hh, sh, s1, s2):
                d = (hh - sh).reshape(GR // 8, 8, D)
                return s1 + jnp.sum(d, axis=0), s2 + jnp.sum(d * d, axis=0)

            h0 = inv(0)
            sh = jnp.sum(jnp.sum(h0.reshape(GR // 8, 8, D), axis=0), axis=0, keepdims=True) * (1.0 / GR)
            zz = jnp.zeros((8, D), f32)
            s1, s2 = acc(h0, sh, zz, zz)
            s1, s2 = jax.lax.fori_loop(1, NG - 1, lambda gi, c: acc(inv(gi), sh, *c), (s1, s2), unroll=NG - 2)
            hl = inv(NG - 1)
            row = jax.lax.broadcasted_iota(jnp.int32, (GR, D), 0)
            d = jnp.where(row < L - GR * (NG - 1), hl - sh, 0.0).reshape(GR // 8, 8, D)
            s1 = s1 + jnp.sum(d, axis=0)
            s2 = s2 + jnp.sum(d * d, axis=0)
            dm = jnp.sum(s1, axis=0, keepdims=True) * (1.0 / L)
            mu = sh + dm
            var = jnp.maximum(jnp.sum(s2, axis=0, keepdims=True) * (1.0 / L) - dm * dm, 0.0)
            scale = g_ref[...].reshape(1, D).astype(f32) / jnp.sqrt(var + 1e-5)
            shift = b_ref[...].reshape(1, D).astype(f32) - mu * scale
            st_ref[0:1, :] = scale
            st_ref[1:2, :] = shift

        @pl.when(step == 0)
        def _():
            def fin0(gi, c):
                y0 = finish(pltpu.bitcast(buf_ref[h_idx(gi)], f32), 0)
                sh_ref[pl.ds(pl.multiple_of(gi * GR, GR), GR), :] = y0.astype(bf16)
                return c
            jax.lax.fori_loop(0, NG, fin0, 0)

        @pl.when(step >= B)
        def _():
            def fin(j, c):
                gi = (step - B) * GPC + j
                y1 = finish(pltpu.bitcast(buf_ref[h_idx(gi)], f32), 0)
                y0 = sh_ref[pl.ds(pl.multiple_of(gi * GR, GR), GR), :]
                y1b = y1.astype(bf16)
                cols = []
                for jj in range(GR // 16):
                    cols.append(jnp.concatenate(
                        [yy[16 * jj:16 * jj + 16, 128 * cc:128 * (cc + 1)] for yy in (y0, y1b) for cc in range(4)], axis=0))
                sm = jnp.concatenate(cols, axis=1)
                r = _dot(pm_ref[...], sm)
                rr = jnp.concatenate([r[:, 128 * jj:128 * (jj + 1)] for jj in range(GR // 16)], axis=0)
                o_ref[pl.ds(pl.multiple_of(j * 8 * GR, 8 * GR), 8 * GR), :] = rr.astype(bf16)
                return c
            jax.lax.fori_loop(0, GPC, fin, 0, unroll=GPC)

    vm = lambda shape: pl.BlockSpec(shape, lambda s: (0,) * len(shape), pipeline_mode=pl.Buffered(1))
    any_spec = pl.BlockSpec(memory_space=pl.ANY)
    out = pl.pallas_call(
        kernel,
        grid=(B + NCH,),
        in_specs=[any_spec, any_spec, vm((D,)), vm((D,)),
                  vm((256, 128)), vm((256, 256)), vm((256, 128)), vm((256, 256)), vm((8 * len(_MXU_COMPS), 128)), vm((128, 128))],
        out_specs=pl.BlockSpec((CH * 8, 128), lambda s: (jnp.maximum(s - B, 0), 0)),
        out_shape=jax.ShapeDtypeStruct((L * 8, 128), x.dtype),
        scratch_shapes=[
            pltpu.VMEM((_NS, 2 * D, 2 * D), bf16),
            pltpu.VMEM((XPAD, D), bf16),
            pltpu.VMEM((_NS * NW, 2 * D), jnp.uint32),
            pltpu.VMEM((_NS, MR, D), bf16),
            pltpu.VMEM((8, D), f32),
            pltpu.VMEM((NG * GR, D), bf16),
            pltpu.SemaphoreType.DMA((3,)),
            pltpu.SemaphoreType.DMA((NWS,)),
        ],
        compiler_params=pltpu.CompilerParams(
            dimension_semantics=("arbitrary",),
            vmem_limit_bytes=128 * 1024 * 1024,
        ),
    )(x, w, gn_gamma, gn_beta, *_CONSTS)
    return out.reshape(L, 4, B, 128).transpose(2, 0, 1, 3).reshape(B, L, D)
```
